```python
import jax
import jax.numpy as jnp

def _softmax(x, axis=-1):
    return jax.nn.softmax(x, axis=axis)

def _gelu(x):
    return jax.nn.gelu(x, approximate=True)

def _silu(x):
    return jax.nn.silu(x)

def _sigmoid(x):
    return jax.nn.sigmoid(x)

def _layernorm(x, axis=-1, eps=1e-05):
    m = jnp.mean(x, axis=axis, keepdims=True)
    v = jnp.var(x, axis=axis, keepdims=True)
    return (x - m) / jnp.sqrt(v + eps)

def _scatter_add(tgt, idx, src, axis=0):
    return tgt.at[idx].add(src)

def _segment_sum(src, seg, n):
    return jax.ops.segment_sum(src, seg, n)

class _Rng:

    def __init__(self, key):
        self._k = key

    def _next(self):
        self._k, sub = jax.random.split(self._k)
        return sub

    def normal(self, shape):
        return jax.random.normal(self._next(), shape, dtype=jnp.bfloat16)

    def randint(self, lo, hi, shape):
        return jax.random.randint(self._next(), shape, lo, hi, dtype=jnp.int32)

    def uniform(self, shape, lo=0.0, hi=1.0):
        return jax.random.uniform(self._next(), shape, jnp.bfloat16, lo, hi)

    def permutation(self, n):
        return jax.random.permutation(self._next(), n)
kernel_name = 'adaLN_cond__compressed_kv_cla__moe_arch_mod__prompt'

def setup_inputs():
    _rng = _Rng(jax.random.key(int.from_bytes(__import__("os").urandom(4), "little")))
    _w = lambda a: (lambda t: t.astype(jnp.bfloat16) if jnp.issubdtype(t.dtype, jnp.floating) else t)(jnp.asarray(a))

    def _A_setup():
        B, H, Sq, Sk, D, M = (1, 32, 2048, 2048, 128, 640)
        Dc = 4 * D
        return {'x': _w((lambda *s: _rng.normal(s) * 0.05)(B, Sq, M)), 'c_kv': _w((lambda *s: _rng.normal(s) * 0.05)(B, Sk, Dc)), 'w_q': _w((lambda *s: _rng.normal(s) * 0.05)(M, H, D) * M ** (-0.5)), 'w_uk': _w((lambda *s: _rng.normal(s) * 0.05)(Dc, H, D) * Dc ** (-0.5)), 'w_uv': _w((lambda *s: _rng.normal(s) * 0.05)(Dc, H, D) * Dc ** (-0.5)), 'w_o': _w((lambda *s: _rng.normal(s) * 0.05)(H, D, M) * (H * D) ** (-0.5))}
    _A_in = _A_setup()

    def _B_setup():
        B, S, D, F, C = (1, 2048, 640, 1728, 8)
        return {'x': _w((lambda *s: _rng.normal(s) * 0.05)(B, S, D)), 'w_r': _w((lambda *s: _rng.normal(s) * 0.05)(D)), 'w_gate': _w((lambda *s: _rng.normal(s) * 0.05)(D, F)), 'w_up': _w((lambda *s: _rng.normal(s) * 0.05)(D, F)), 'w_down': _w((lambda *s: _rng.normal(s) * 0.05)(F, D))}
    _B_in = _B_setup()
    return {'A_x': _A_in['x'], 'A_c_kv': _A_in['c_kv'], 'A_w_q': _A_in['w_q'], 'A_w_uk': _A_in['w_uk'], 'A_w_uv': _A_in['w_uv'], 'A_w_o': _A_in['w_o'], 'B_x': _B_in['x'], 'B_w_r': _B_in['w_r'], 'B_w_gate': _B_in['w_gate'], 'B_w_up': _B_in['w_up'], 'B_w_down': _B_in['w_down'], 'c': _w((lambda *s: _rng.normal(s) * 0.05)(1, 640)), 'w_mod': _w((lambda *s: _rng.normal(s) * 0.05)(640, 6 * 640) * 640 ** (-0.5))}

def reference(A_x, A_c_kv, A_w_q, A_w_uk, A_w_uv, A_w_o, B_x, B_w_r, B_w_gate, B_w_up, B_w_down, c, w_mod):

    def _A_ref(x, c_kv, w_q, w_uk, w_uv, w_o):
        B, Sq, M = (x.shape[0], x.shape[1], x.shape[2])
        Sk = c_kv.shape[1]
        H, D = (w_q.shape[1], w_q.shape[2])
        q = jnp.einsum('bqm,mhd->bhqd', x, w_q)
        k = jnp.einsum('bkc,chd->bhkd', c_kv, w_uk)
        v = jnp.einsum('bkc,chd->bhkd', c_kv, w_uv)
        scores = jnp.einsum('bhqd,bhkd->bhqk', q, k) * D ** (-0.5)
        off = Sk - Sq
        qi = jnp.arange(Sq)[:, None]
        kj = jnp.arange(Sk)[None, :]
        cmask = kj <= qi + off
        scores = jnp.where(cmask[None, None], scores, -1000000000.0)
        p = _softmax(scores, axis=-1)
        ctx = jnp.einsum('bhqk,bhkd->bhqd', p, v)
        return jnp.einsum('bhqd,hdm->bqm', ctx, w_o)

    def _B_ref(x, w_r, w_gate, w_up, w_down):
        B, S, D = x.shape
        C = 8
        r = x @ w_r
        idx = jnp.argsort(-r, axis=-1)[:, :C]
        idx_e = jnp.repeat(idx.reshape(B, C, 1), D, axis=2)
        x_sel = jnp.take_along_axis(x, idx_e, axis=1)
        g = _silu(x_sel @ w_gate)
        u = x_sel @ w_up
        y = g * u @ w_down
        r_sel = _sigmoid(jnp.take_along_axis(r, idx, axis=1))
        y = y * r_sel.reshape(B, C, 1)
        b_off = (jnp.arange(B) * S).reshape(B, 1)
        flat_idx = (idx + b_off).reshape(B * C)
        zero = (x * 0.0).reshape(B * S, D)
        upd = _scatter_add(zero, flat_idx, y.reshape(B * C, D), axis=0)
        return x + upd.reshape(B, S, D)
    x = A_x
    mod = (_silu(c) @ w_mod).reshape(c.shape[0], 6, 1, -1)
    sa, ca, ga, sb, cb, gb = (mod[:, 0].copy(), mod[:, 1].copy(), mod[:, 2].copy(), mod[:, 3].copy(), mod[:, 4].copy(), mod[:, 5].copy())
    h = _layernorm(x, axis=-1) * (1 + ca) + sa
    x = x + ga * _A_ref(h, A_c_kv, A_w_q, A_w_uk, A_w_uv, A_w_o)
    h = _layernorm(x, axis=-1) * (1 + cb) + sb
    x = x + gb * _B_ref(h, B_w_r, B_w_gate, B_w_up, B_w_down)
    return x
```

```python
import math

import jax
import jax.numpy as jnp
from jax import lax
import jax.experimental.pallas as pl
import jax.experimental.pallas.tpu as pltpu

F32 = jnp.float32
BF16 = jnp.bfloat16
U32 = jnp.uint32
I32 = jnp.int32

TOPK = 8
EPS = 1e-05
LOG2E = math.log2(math.e)
MASK_LOG2 = -1000000000.0 * LOG2E
BQ = 128
HEADS_PER_ITER = 2
ROWS_C = 256
NT = (((1,), (1,)), ((), ()))


def _r(x):
    return x.astype(BF16).astype(F32)


def _dot(a, b):
    return jnp.dot(a, b, preferred_element_type=F32)


def _dot_nt(a, b):
    return lax.dot_general(a, b, NT, preferred_element_type=F32)


def _split_pair(raw):
    n = raw.shape[0]
    w = pltpu.bitcast(raw.reshape(2 * n, raw.shape[2]), U32)
    lo = pltpu.bitcast(w << 16, F32).astype(BF16)
    hi = pltpu.bitcast(w & jnp.uint32(0xFFFF0000), F32).astype(BF16)
    return lo, hi


def _modulated_ln(x, shift, scale1):
    inv_n = 1.0 / x.shape[-1]
    mean = jnp.sum(x, axis=-1, keepdims=True) * inv_n
    xc = x - mean
    var = jnp.sum(xc * xc, axis=-1, keepdims=True) * inv_n
    std = _r(jnp.sqrt(_r(_r(var) + EPS)))
    n = _r(_r(x - _r(mean)) / std)
    return _r(_r(n * scale1) + shift)


def _kernel(x_hbm, ckv_hbm, wq_hbm, wuk_hbm, wuv_hbm, wo_hbm, wr_ref, wgt_hbm,
            wut_hbm, wd_hbm, c_ref, wmod_hbm, out_hbm,
            x_v, ckv_v, wq_raw, wk_raw, wv_raw, wo_v, wgt_v, wut_v, wd_v, wmod_v,
            mod_v, h_v, wq_v, wkv_v, k_v, v_v, q_v, ctx_v, out_v,
            sem_w, sem_in, sem_out, sem_fix):
    S, M = x_v.shape
    DC = ckv_v.shape[1]
    H = k_v.shape[0]
    D = k_v.shape[2]
    NP = H // 2
    NB = S // BQ

    def w_copy(j, p):
        src, dst = ((wuk_hbm, wk_raw), (wuv_hbm, wv_raw), (wq_hbm, wq_raw))[j]
        start = 2 * p if isinstance(p, int) else pl.multiple_of(2 * p, 2)
        return pltpu.make_async_copy(src.at[:, pl.ds(start, 2), :], dst.at[p],
                                     sem_w.at[j, p])

    cp_ckv = pltpu.make_async_copy(ckv_hbm, ckv_v, sem_in.at[0])
    cp_x = pltpu.make_async_copy(x_hbm, x_v, sem_in.at[1])
    cp_wmod = pltpu.make_async_copy(wmod_hbm, wmod_v, sem_in.at[2])
    cp_wo = pltpu.make_async_copy(wo_hbm, wo_v, sem_in.at[3])
    cp_wg = pltpu.make_async_copy(wgt_hbm, wgt_v, sem_in.at[4])
    cp_wu = pltpu.make_async_copy(wut_hbm, wut_v, sem_in.at[5])
    cp_wd = pltpu.make_async_copy(wd_hbm, wd_v, sem_in.at[6])

    w_copy(0, 0).start()
    w_copy(1, 0).start()
    cp_ckv.start()
    w_copy(0, 1).start()
    w_copy(1, 1).start()
    w_copy(2, 0).start()

    def stage_kv_weights(p, slot):
        k0, k1 = _split_pair(wk_raw[p])
        v0, v1 = _split_pair(wv_raw[p])
        wkv_v[slot] = jnp.concatenate([k0, k1, v0, v1], axis=1)

    w_copy(0, 0).wait()
    w_copy(1, 0).wait()
    stage_kv_weights(0, 0)
    for p in range(2, NP):
        w_copy(0, p).start()
        w_copy(1, p).start()
        w_copy(2, p - 1).start()
    w_copy(2, NP - 1).start()
    cp_wmod.start()
    cp_x.start()
    cp_ckv.wait()

    def kv_proj(p, stage_next=True):
        slot = p % 2
        if stage_next:
            w_copy(0, p + 1).wait()
            w_copy(1, p + 1).wait()
        w_copy(2, p).wait()
        kv = _dot(ckv_v[...], wkv_v[slot]).astype(BF16)
        k_v[2 * p] = kv[:, 0 * D:1 * D]
        k_v[2 * p + 1] = kv[:, 1 * D:2 * D]
        v_v[2 * p] = kv[:, 2 * D:3 * D]
        v_v[2 * p + 1] = kv[:, 3 * D:4 * D]
        if stage_next:
            stage_kv_weights(p + 1, 1 - slot)
        q0, q1 = _split_pair(wq_raw[p])
        wq_v[2 * p] = q0
        wq_v[2 * p + 1] = q1

    def modulation():
        cf = c_ref[...].astype(F32)
        s = _r(cf * jax.nn.sigmoid(cf))
        s_col = jnp.broadcast_to(s, (128, M)).T
        for j in range(wmod_v.shape[1] // 128):
            w = wmod_v[:, j * 128:(j + 1) * 128].astype(F32)
            col = _r(jnp.sum(w * s_col, axis=0, keepdims=True))
            mod_v[:, j * 128:(j + 1) * 128] = jnp.broadcast_to(col, (8, 128))

    def mod_row(i):
        return mod_v[0:1, i * M:(i + 1) * M]

    def ln1(r0, rows):
        xf = x_v[pl.ds(r0, rows), :].astype(F32)
        h = _modulated_ln(xf, mod_row(0), _r(1.0 + mod_row(1)))
        h_v[pl.ds(r0, rows), :] = h.astype(BF16)

    n_ln = 8
    p_mod = NP - n_ln - 2
    ln_rows = S // n_ln

    def a1(p, carry):
        kv_proj(p)
        return carry

    lax.fori_loop(0, p_mod, a1, 0)
    cp_wmod.wait()
    cp_x.wait()
    cp_wo.start()
    cp_wg.start()
    cp_wu.start()
    cp_wd.start()
    kv_proj(p_mod)
    modulation()

    def a2(t, carry):
        kv_proj(p_mod + 1 + t)
        ln1(pl.multiple_of(t * ln_rows, ln_rows), ln_rows)
        return carry

    lax.fori_loop(0, n_ln, a2, 0)
    kv_proj(NP - 1, stage_next=False)

    qscale = D ** (-0.5) * LOG2E

    def heads_body(it, carry):
        row = lax.broadcasted_iota(I32, (BQ, BQ), 0)
        col = lax.broadcasted_iota(I32, (BQ, BQ), 1)
        causal = col <= row

        def q_proj(u, i):
            h = it * HEADS_PER_ITER + u
            q = _dot(h_v[i * BQ:(i + 1) * BQ, :], wq_v[h]) * qscale
            q_v[u, i * BQ:(i + 1) * BQ, :] = q.astype(BF16)

        def qk(u, i):
            h = it * HEADS_PER_ITER + u
            kend = (i + 1) * BQ
            s = _dot_nt(q_v[u, i * BQ:(i + 1) * BQ, :], k_v[h, :kend, :])
            sd = jnp.where(causal, s[:, kend - BQ:], MASK_LOG2)
            s = jnp.concatenate([s[:, :kend - BQ], sd], axis=1) if i else sd
            return s, jnp.max(s, axis=1, keepdims=True)

        def pv(u, i, s, m, prev_inv):
            h = it * HEADS_PER_ITER + u
            kend = (i + 1) * BQ
            if prev_inv is not None:
                m = jnp.where(prev_inv < 0.0, prev_inv, m)
            p = jnp.exp2(s - m)
            inv = 1.0 / jnp.sum(p, axis=1, keepdims=True)
            o = _dot(p.astype(BF16), v_v[h, :kend, :])
            ctx_v[h, i * BQ:(i + 1) * BQ, :] = (o * inv).astype(BF16)
            return inv

        steps = [(u, i) for u in range(HEADS_PER_ITER) for i in range(NB)]
        n = len(steps)
        q_proj(*steps[0])
        q_proj(*steps[1])
        cur = qk(*steps[0])
        invs = []
        for t in range(n):
            if t + 2 < n:
                q_proj(*steps[t + 2])
            nxt = qk(*steps[t + 1]) if t + 1 < n else None
            invs.append(pv(*steps[t], *cur, invs[t - 2] if t >= 2 else None))
            cur = nxt
        return carry

    lax.fori_loop(0, H // HEADS_PER_ITER, heads_body, 0)

    cp_wo.wait()
    wr = wr_ref[...].astype(F32).reshape(1, M)
    n_c = S // ROWS_C

    def out_copy(t):
        r0 = t * ROWS_C if isinstance(t, int) else pl.multiple_of(t * ROWS_C, ROWS_C)
        return pltpu.make_async_copy(out_v.at[pl.ds(r0, ROWS_C), :],
                                     out_hbm.at[pl.ds(r0, ROWS_C), :], sem_out.at[t])

    def c_body(t, scores):
        lane = lax.broadcasted_iota(I32, (8, S // 8), 1)
        for b in range(ROWS_C // BQ):
            r0 = pl.multiple_of(t * ROWS_C + b * BQ, BQ)
            rows = pl.ds(r0, BQ)
            ctx = jnp.concatenate([ctx_v[h, rows, :] for h in range(H)], axis=1)
            attn = _r(_dot(ctx, wo_v[...]))
            x1 = _r(x_v[rows, :].astype(F32) + _r(mod_row(2) * attn))
            h2 = _modulated_ln(x1, mod_row(3), _r(1.0 + mod_row(4)))
            out = x1 + _r(mod_row(5) * (h2 + h2 * 0.0))
            x_v[rows, :] = x1.astype(BF16)
            h_v[rows, :] = h2.astype(BF16)
            out_v[rows, :] = out.astype(BF16)
            r = jnp.sum(h2 * wr, axis=1, keepdims=True)
            for g in range(BQ // 8):
                scores = jnp.where(lane == r0 // 8 + g, r[g * 8:(g + 1) * 8], scores)
        out_copy(t).start()
        return scores

    scores = lax.fori_loop(0, n_c, c_body, jnp.zeros((8, S // 8), F32))

    rb = _r(scores)
    bits = pltpu.bitcast(jnp.where(rb == 0.0, 0.0, rb), I32)
    k16 = (bits >> 16) & 0xFFFF
    k16 = jnp.where(bits < 0, 0xFFFF - k16, k16 + 0x8000)
    k16 = jnp.where(rb != rb, 0, k16)
    ridx = (lax.broadcasted_iota(I32, scores.shape, 1) * 8
            + lax.broadcasted_iota(I32, scores.shape, 0))
    idx_bits = (S - 1).bit_length()
    key = pltpu.bitcast((k16 << idx_bits) + (S - 1 - ridx) + (1 << 29), F32)
    picks = []
    for _ in range(TOPK):
        top = jnp.max(jnp.max(key, axis=1, keepdims=True), axis=0, keepdims=True)
        key = jnp.where(key == top, 1.0e-30, key)
        picks.append(S - 1 - (pltpu.bitcast(top, I32)[0, 0] & ((1 << idx_bits) - 1)))

    row16 = lax.broadcasted_iota(I32, (16, M), 0)

    def tile_of(i):
        return pl.ds(pl.multiple_of((i // 16) * 16, 16), 16)

    sel = jnp.zeros((16, M), F32)
    for j, i in enumerate(picks):
        tile = h_v[tile_of(i), :].astype(F32)
        hrow = jnp.sum(jnp.where(row16 == i % 16, tile, 0.0), axis=0, keepdims=True)
        sel = jnp.where(row16 == j, hrow, sel)

    cp_wg.wait()
    cp_wu.wait()
    cp_wd.wait()
    sel_b = sel.astype(BF16)
    g = _r(_dot_nt(sel_b, wgt_v[...]))
    g = _r(g * jax.nn.sigmoid(g))
    u = _r(_dot_nt(sel_b, wut_v[...]))
    y = _r(_dot((g * u).astype(BF16), wd_v[...]))
    gate = _r(jax.nn.sigmoid(_r(jnp.sum(sel * wr, axis=1, keepdims=True))))
    y = _r(y * gate)
    delta = _r(mod_row(5) * _r(sel + _r(sel * 0.0 + y)))

    for t in range(n_c):
        out_copy(t).wait()
    for j, i in enumerate(picks):
        new = (x_v[tile_of(i), :].astype(F32) + delta[j:j + 1, :]).astype(BF16)
        out_v[tile_of(i), :] = jnp.where(row16 == i % 16, new, out_v[tile_of(i), :])

    def fix_copy(j):
        return pltpu.make_async_copy(out_v.at[tile_of(picks[j]), :],
                                     out_hbm.at[tile_of(picks[j]), :], sem_fix.at[j])

    first = []
    for j in range(TOPK):
        f = jnp.bool_(True)
        for e in range(j):
            f = jnp.logical_and(f, picks[e] // 16 != picks[j] // 16)
        first.append(f)
    for j in range(TOPK):
        pl.when(first[j])(fix_copy(j).start)
    for j in range(TOPK):
        pl.when(first[j])(fix_copy(j).wait)


@jax.jit
def pallas_adaLN_cond__compressed_kv_cla__moe_arch_mod__prompt_kernel(
    A_x: jax.Array,
    A_c_kv: jax.Array,
    A_w_q: jax.Array,
    A_w_uk: jax.Array,
    A_w_uv: jax.Array,
    A_w_o: jax.Array,
    B_x: jax.Array,
    B_w_r: jax.Array,
    B_w_gate: jax.Array,
    B_w_up: jax.Array,
    B_w_down: jax.Array,
    c: jax.Array,
    w_mod: jax.Array,
):
    del B_x
    _, S, M = A_x.shape
    DC = A_c_kv.shape[2]
    _, H, D = A_w_q.shape
    F = B_w_gate.shape[1]
    NP = H // 2

    hbm = pl.BlockSpec(memory_space=pl.ANY)
    vmem = pl.BlockSpec(memory_space=pltpu.VMEM)
    scratch = [
        pltpu.VMEM((S, M), BF16),
        pltpu.VMEM((S, DC), BF16),
        pltpu.VMEM((NP, M, 2, D), BF16),
        pltpu.VMEM((NP, DC, 2, D), BF16),
        pltpu.VMEM((NP, DC, 2, D), BF16),
        pltpu.VMEM((H * D, M), BF16),
        pltpu.VMEM((F, M), BF16),
        pltpu.VMEM((F, M), BF16),
        pltpu.VMEM((F, M), BF16),
        pltpu.VMEM((M, 6 * M), BF16),
        pltpu.VMEM((8, 6 * M), F32),
        pltpu.VMEM((S, M), BF16),
        pltpu.VMEM((H, M, D), BF16),
        pltpu.VMEM((2, DC, 4 * D), BF16),
        pltpu.VMEM((H, S, D), BF16),
        pltpu.VMEM((H, S, D), BF16),
        pltpu.VMEM((HEADS_PER_ITER, S, D), BF16),
        pltpu.VMEM((H, S, D), BF16),
        pltpu.VMEM((S, M), BF16),
        pltpu.SemaphoreType.DMA((3, NP)),
        pltpu.SemaphoreType.DMA((7,)),
        pltpu.SemaphoreType.DMA((S // ROWS_C,)),
        pltpu.SemaphoreType.DMA((TOPK,)),
    ]
    out = pl.pallas_call(
        _kernel,
        in_specs=[hbm, hbm, hbm, hbm, hbm, hbm, vmem, hbm, hbm, hbm, vmem, hbm],
        out_specs=hbm,
        out_shape=jax.ShapeDtypeStruct((S, M), A_x.dtype),
        scratch_shapes=scratch,
        compiler_params=pltpu.CompilerParams(vmem_limit_bytes=124 * 1024 * 1024),
        name="adaln_cla_moe",
    )(A_x.reshape(S, M), A_c_kv.reshape(S, DC), A_w_q, A_w_uk, A_w_uv,
      A_w_o.reshape(H * D, M), B_w_r, B_w_gate.T, B_w_up.T, B_w_down, c, w_mod)
    return out.reshape(A_x.shape)
```

```python
import functools
import math

import jax
import jax.numpy as jnp
from jax import lax
import jax.experimental.pallas as pl
import jax.experimental.pallas.tpu as pltpu

F32 = jnp.float32
BF16 = jnp.bfloat16
U32 = jnp.uint32
I32 = jnp.int32

TOPK = 8
EPS = 1e-05
LOG2E = math.log2(math.e)
MASK_LOG2 = -1000000000.0 * LOG2E
BQ = 128
HG = 8
A_STEPS = 4
HEADS_PER_ITER = 2
SUB_C = 2
LN_ROWS = 16
ST_ROWS = 16
LN1_GAP = 2
LN2_GAP = 3
END_GAP = 2
NT = (((1,), (1,)), ((), ()))


def _r(x):
    return x.astype(BF16).astype(F32)


def _dot(a, b):
    return jnp.dot(a, b, preferred_element_type=F32)


def _dot_nt(a, b):
    return lax.dot_general(a, b, NT, preferred_element_type=F32)


def _pack(x):
    return pltpu.bitcast(x.astype(BF16), U32)


def _unpack(x):
    return pltpu.bitcast(x, BF16)


def _ds(start, size):
    if not isinstance(start, int):
        start = pl.multiple_of(start, size)
    return pl.ds(start, size)


class _Pacer:
    def __init__(self):
        self.word = None

    def tick(self, x, gap=1):
        x = pltpu.bitcast(x, U32)
        tiles = [x[r:r + 8, c:c + 128]
                 for r in range(0, x.shape[0], 8) for c in range(0, x.shape[1], 128)]
        word = functools.reduce(jnp.bitwise_or, tiles)
        self.word = word if self.word is None else self.word | word
        self.idle(gap)

    def idle(self, gap):
        for _ in range(gap):
            self.word = pltpu.roll(self.word, 1, 1)


def _modulated_ln(x, shift, scale1):
    inv_n = 1.0 / x.shape[-1]
    mean = jnp.sum(x, axis=-1, keepdims=True) * inv_n
    xc = x - mean
    var = jnp.sum(xc * xc, axis=-1, keepdims=True) * inv_n
    std = _r(jnp.sqrt(_r(_r(var) + EPS)))
    n = _r(_r(x - _r(mean)) / std)
    return _r(_r(n * scale1) + shift)


def _kernel(x_hbm, ckv_hbm, wq_hbm, wuk_hbm, wuv_hbm, wo_hbm, wr_ref, wgt_hbm,
            wut_hbm, wd_hbm, c_ref, wmod_hbm, out_hbm,
            x_v, ckv_v, wq_raw, wkv_raw, wo_v, wgt_v, wut_v, wd_v, wmod_v,
            a_v, h_v, kv_v, ctx_v, x1_v, h2_v, out_v, pend_v, scol_v, mod_v,
            sem_kv, sem_ckv, sem_q, sem_mod, sem_in, sem_out, sem_fix):
    S, M = x_v.shape
    DC = ckv_v.shape[1]
    H, _, D = ctx_v.shape
    NG = H // HG
    NB = S // BQ
    B2 = BQ // 2
    NA = 4 * NG
    NM = M // 128
    NL = NA // 2
    N0 = NA - NL - NM
    WQ0, MOD0 = 4, 4 + 2 * NM

    def kv_copy(n):
        g, rows = n // 2, pl.ds((n % 2) * (DC // 2), DC // 2)
        src = wuk_hbm if g < NG else wuv_hbm
        return pltpu.make_async_copy(src.at[rows, pl.ds((g % NG) * HG, HG), :],
                                     wkv_raw.at[g, rows], sem_kv.at[n])

    def q_copy(g):
        return pltpu.make_async_copy(wq_hbm.at[:, pl.ds(g * HG, HG), :], wq_raw.at[g],
                                     sem_q.at[g])

    def row_copy(src, dst, sems, n, j):
        rows = pl.ds(j * n, n)
        return pltpu.make_async_copy(src.at[rows], dst.at[rows], sems.at[j])

    ckv_copy = functools.partial(row_copy, ckv_hbm, ckv_v, sem_ckv, S // 2)
    mod_copy = functools.partial(row_copy, wmod_hbm, wmod_v, sem_mod, 128)
    cp_x = pltpu.make_async_copy(x_hbm, x_v, sem_in.at[0])
    cp_wo = pltpu.make_async_copy(wo_hbm, wo_v, sem_in.at[1])
    cp_wg = pltpu.make_async_copy(wgt_hbm, wgt_v, sem_in.at[2])
    cp_wu = pltpu.make_async_copy(wut_hbm, wut_v, sem_in.at[3])
    cp_wd = pltpu.make_async_copy(wd_hbm, wd_v, sem_in.at[4])

    needs = []
    for n in range(NA):
        cps = [ckv_copy(n)] if n < 2 else []
        if n + 2 < NA:
            cps.append(kv_copy(n + 2))
        if N0 <= n < N0 + NM:
            cps.append(mod_copy(n - N0))
        if n == N0:
            cps += [q_copy(g) for g in range(NG)]
        if n == N0 + NM:
            cps.append(cp_x)
        needs.append(cps)

    needs += [[cp_wo], [cp_wg, cp_wu, cp_wd]]
    kv_copy(0).start()
    kv_copy(1).start()
    for cp in needs[0]:
        cp.start()

    cf = c_ref[...].astype(F32)
    scol_v[...] = jnp.broadcast_to(_r(cf * jax.nn.sigmoid(cf)), (128, M)).T
    pend_v[...] = jnp.zeros(pend_v.shape, F32)

    def stage_kv(n, lo, rows):
        src = jnp.minimum(n, NA - 1)
        w = wkv_raw[src // 2, _ds((src % 2) * (DC // 2) + lo, rows)]
        w = _pack(w.reshape(rows, HG * D))
        a_v[n % 4, lo // 2:(lo + rows) // 2, :] = w
        return w

    for n in range(2):
        kv_copy(n).wait()
        stage_kv(n, 0, DC // 2)

    def kv_loop(lo, hi, side_job):
        rows = S // 2 // A_STEPS

        def body(n, carry):
            for k in range(lo, hi):
                @pl.when(n == k)
                def _(k=k):
                    for cp in needs[k]:
                        cp.wait()
                    for cp in (needs[1] if k == 0 else []) + needs[k + 2]:
                        cp.start()

            g, half = n // 2, n % 2
            for st in range(A_STEPS):
                r0 = half * (S // 2) + st * rows
                w = jnp.concatenate([a_v[2 * (g % 2)], a_v[2 * (g % 2) + 1]], axis=0)
                kv = _pack(_dot(ckv_v[_ds(r0, rows), :], _unpack(w)))
                for j in range(HG):
                    kv_v[g * HG + j, _ds(r0 // 2, rows // 2), :] = kv[:, j * D:(j + 1) * D]
            pacer = _Pacer()
            for r in range(0, DC // 2, ST_ROWS):
                pacer.tick(stage_kv(n + 2, r, ST_ROWS))
            side_job(n - lo, pacer)
            pacer.idle(END_GAP)
            a_v[MOD0, 64:72, 0:128] = pacer.word
            return carry

        lax.fori_loop(lo, hi, body, 0)

    def mod_and_wq(t, pacer):
        rows = _ds(t * 128, 128)
        tiles = [(i, j) for i in range(6) for j in range(M // 128)]
        for g in range(NG):
            for r in range(0, 128, ST_ROWS):
                if tiles:
                    i, j = tiles.pop(0)
                    prod = wmod_v[rows, i * M + j * 128:i * M + (j + 1) * 128].astype(F32)
                    prod = prod * scol_v[rows, :]
                    acc = functools.reduce(jnp.add, [prod[e:e + 8] for e in range(0, 128, 8)])
                    a_v[MOD0 + t, i * 8:(i + 1) * 8, j * 128:(j + 1) * 128] = (
                        pltpu.bitcast(acc, U32))
                    pacer.tick(acc, 0)
                w = _pack(wq_raw[g, _ds(t * 128 + r, ST_ROWS)].reshape(ST_ROWS, HG * D))
                r0 = (g % 2) * 64 + r // 2
                a_v[WQ0 + 2 * t + g // 2, r0:r0 + ST_ROWS // 2, :] = w
                pacer.tick(w)
        assert not tiles

    def mod_row(i):
        return mod_v[i, 0:1, :]

    def ln1(t, pacer):
        for e in range(S // NL // LN_ROWS):
            r0 = t * (S // NL) + e * LN_ROWS
            xf = x_v[_ds(r0, LN_ROWS), :].astype(F32)
            h = _pack(_modulated_ln(xf, mod_row(0), mod_row(1)))
            h_v[_ds(r0 // 2, LN_ROWS // 2), :] = h
            pacer.tick(h, LN1_GAP)

    kv_loop(0, N0, lambda t, pacer: None)
    kv_loop(N0, N0 + NM, mod_and_wq)
    for i in range(6):
        parts = [pltpu.bitcast(a_v[MOD0 + t, i * 8:(i + 1) * 8, :M], F32)
                 for t in range(NM)]
        mod = _r(jnp.sum(functools.reduce(jnp.add, parts), axis=0, keepdims=True))
        if i % 3 == 1:
            mod = _r(1.0 + mod)
        mod_v[i] = jnp.broadcast_to(mod, (8, M))
    kv_loop(N0 + NM, NA, ln1)

    qscale = D ** (-0.5) * LOG2E

    def heads_body(it, carry):
        row = lax.broadcasted_iota(I32, (BQ, BQ), 0)
        col = lax.broadcasted_iota(I32, (BQ, BQ), 1)
        causal = col <= row
        qs = {}

        def q_proj(u, i):
            h = it * HEADS_PER_ITER + u
            g = h // HG
            w = jnp.concatenate(
                [a_v[WQ0 + 2 * t + g // 2, _ds((g % 2) * 64, 64), _ds((h % HG) * D, D)]
                 for t in range(NM)], axis=0)
            q = _dot(_unpack(h_v[i * B2:(i + 1) * B2, :]), _unpack(w)) * qscale
            qs[u, i] = q.astype(BF16)

        def qk(u, i):
            h = it * HEADS_PER_ITER + u
            kend = (i + 1) * BQ
            s = _dot_nt(qs[u, i], _unpack(kv_v[h, :kend // 2, :]))
            sd = jnp.where(causal, s[:, kend - BQ:], MASK_LOG2)
            s = jnp.concatenate([s[:, :kend - BQ], sd], axis=1) if i else sd
            return s, jnp.max(s, axis=1, keepdims=True)

        def pv(u, i, s, m, prev_inv):
            h = it * HEADS_PER_ITER + u
            kend = (i + 1) * BQ
            if prev_inv is not None:
                m = jnp.where(prev_inv < 0.0, prev_inv, m)
            p = jnp.exp2(s - m)
            inv = 1.0 / jnp.sum(p, axis=1, keepdims=True)
            o = _dot(p.astype(BF16), _unpack(kv_v[H + h, :kend // 2, :]))
            ctx_v[h, i * B2:(i + 1) * B2, :] = _pack(o * inv)
            return inv

        steps = [(u, i) for u in range(HEADS_PER_ITER) for i in range(NB)]
        n = len(steps)
        q_proj(*steps[0])
        q_proj(*steps[1])
        cur = qk(*steps[0])
        inv = None
        for t in range(n):
            if t + 2 < n:
                q_proj(*steps[t + 2])
            nxt = qk(*steps[t + 1]) if t + 1 < n else None
            inv = pv(*steps[t], *cur, inv)
            cur = nxt
        return carry

    lax.fori_loop(0, H // HEADS_PER_ITER, heads_body, 0)

    cp_wo.wait()
    wr = wr_ref[...].astype(F32).reshape(1, M)

    def out_copy(blk):
        return pltpu.make_async_copy(out_v.at[_ds(blk * BQ, BQ), :],
                                     out_hbm.at[_ds(blk * BQ, BQ), :], sem_out.at[blk])

    def finish_rows(attn, r0, scores):
        n = attn.shape[0]
        rows = _ds(r0, n)
        x1 = _r(x_v[rows, :].astype(F32) + _r(mod_row(2) * _r(attn)))
        h2 = _modulated_ln(x1, mod_row(3), mod_row(4))
        out = x1 + _r(mod_row(5) * (h2 + h2 * 0.0))
        x1_v[rows, :] = x1.astype(BF16)
        h2_v[rows, :] = h2.astype(BF16)
        out = out.astype(BF16)
        out_v[rows, :] = out
        r = jnp.sum(h2 * wr, axis=1, keepdims=True)
        lane = lax.broadcasted_iota(I32, scores.shape, 1)
        for g in range(n // 8):
            scores = jnp.where(lane == r0 // 8 + g, r[g * 8:(g + 1) * 8], scores)
        return scores, out

    def c_body(t, scores):
        prev_blk = jnp.maximum(t * SUB_C - 1, 0)
        attn = pend_v[...]
        pacer = _Pacer()
        for b in range(SUB_C):
            blk = t * SUB_C + b
            for lo in range(0, BQ, LN_ROWS):
                scores, out = finish_rows(attn[lo:lo + LN_ROWS], prev_blk * BQ + lo, scores)
                pacer.tick(scores, 0)
                pacer.tick(out, LN2_GAP)
            ctx = jnp.concatenate([ctx_v[h, _ds(blk * B2, B2), :] for h in range(H)], axis=1)
            attn = _dot(_unpack(ctx), wo_v[...])
            prev_blk = blk
        pend_v[...] = attn
        a_v[MOD0, 64:72, 0:128] = pacer.word

        @pl.when(t > 0)
        def _():
            out_copy(t * SUB_C - 1).start()

        for b in range(SUB_C - 1):
            out_copy(t * SUB_C + b).start()
        return scores

    scores = jnp.zeros((8, S // 8), F32)
    scores = lax.fori_loop(0, NB // SUB_C, c_body, scores)
    scores, _ = finish_rows(pend_v[...], (NB - 1) * BQ, scores)
    out_copy(NB - 1).start()

    rb = _r(scores)
    bits = pltpu.bitcast(jnp.where(rb == 0.0, 0.0, rb), I32)
    k16 = (bits >> 16) & 0xFFFF
    k16 = jnp.where(bits < 0, 0xFFFF - k16, k16 + 0x8000)
    k16 = jnp.where(rb != rb, 0, k16)
    ridx = (lax.broadcasted_iota(I32, scores.shape, 1) * 8
            + lax.broadcasted_iota(I32, scores.shape, 0))
    idx_bits = (S - 1).bit_length()
    key = pltpu.bitcast((k16 << idx_bits) + (S - 1 - ridx) + (1 << 29), F32)
    picks = []
    for _ in range(TOPK):
        top = jnp.max(jnp.max(key, axis=1, keepdims=True), axis=0, keepdims=True)
        key = jnp.where(key == top, 1.0e-30, key)
        picks.append(S - 1 - (pltpu.bitcast(top, I32)[0, 0] & ((1 << idx_bits) - 1)))

    row16 = lax.broadcasted_iota(I32, (16, M), 0)

    def tile_of(i):
        return _ds((i // 16) * 16, 16)

    sel = jnp.zeros((16, M), F32)
    for j, i in enumerate(picks):
        tile = h2_v[tile_of(i), :].astype(F32)
        hrow = jnp.sum(jnp.where(row16 == i % 16, tile, 0.0), axis=0, keepdims=True)
        sel = jnp.where(row16 == j, hrow, sel)

    cp_wg.wait()
    cp_wu.wait()
    cp_wd.wait()
    sel_b = sel.astype(BF16)
    g = _r(_dot_nt(sel_b, wgt_v[...]))
    g = _r(g * jax.nn.sigmoid(g))
    u = _r(_dot_nt(sel_b, wut_v[...]))
    y = _r(_dot((g * u).astype(BF16), wd_v[...]))
    gate = _r(jax.nn.sigmoid(_r(jnp.sum(sel * wr, axis=1, keepdims=True))))
    y = _r(y * gate)
    delta = _r(mod_row(5) * _r(sel + _r(sel * 0.0 + y)))

    for t in range(NB):
        out_copy(t).wait()
    for j, i in enumerate(picks):
        new = (x1_v[tile_of(i), :].astype(F32) + delta[j:j + 1, :]).astype(BF16)
        out_v[tile_of(i), :] = jnp.where(row16 == i % 16, new, out_v[tile_of(i), :])

    def fix_copy(j):
        return pltpu.make_async_copy(out_v.at[tile_of(picks[j]), :],
                                     out_hbm.at[tile_of(picks[j]), :], sem_fix.at[j])

    first = []
    for j in range(TOPK):
        f = jnp.bool_(True)
        for e in range(j):
            f = jnp.logical_and(f, picks[e] // 16 != picks[j] // 16)
        first.append(f)
    for j in range(TOPK):
        pl.when(first[j])(fix_copy(j).start)
    for j in range(TOPK):
        pl.when(first[j])(fix_copy(j).wait)


@jax.jit
def pallas_adaLN_cond__compressed_kv_cla__moe_arch_mod__prompt_kernel(
    A_x: jax.Array,
    A_c_kv: jax.Array,
    A_w_q: jax.Array,
    A_w_uk: jax.Array,
    A_w_uv: jax.Array,
    A_w_o: jax.Array,
    B_x: jax.Array,
    B_w_r: jax.Array,
    B_w_gate: jax.Array,
    B_w_up: jax.Array,
    B_w_down: jax.Array,
    c: jax.Array,
    w_mod: jax.Array,
):
    del B_x
    _, S, M = A_x.shape
    DC = A_c_kv.shape[2]
    _, H, D = A_w_q.shape
    F = B_w_gate.shape[1]
    NG = H // HG

    hbm = pl.BlockSpec(memory_space=pl.ANY)
    vmem = pl.BlockSpec(memory_space=pltpu.VMEM)
    scratch = [
        pltpu.VMEM((S, M), BF16),
        pltpu.VMEM((S, DC), BF16),
        pltpu.VMEM((NG, M, HG, D), BF16),
        pltpu.VMEM((2 * NG, DC, HG, D), BF16),
        pltpu.VMEM((H * D, M), BF16),
        pltpu.VMEM((F, M), BF16),
        pltpu.VMEM((F, M), BF16),
        pltpu.VMEM((F, M), BF16),
        pltpu.VMEM((M, 6 * M), BF16),
        pltpu.VMEM((4 + 3 * (M // 128), DC // 4, HG * D), U32),
        pltpu.VMEM((S // 2, M), U32),
        pltpu.VMEM((2 * H, S // 2, D), U32),
        pltpu.VMEM((H, S // 2, D), U32),
        pltpu.VMEM((S, M), BF16),
        pltpu.VMEM((S, M), BF16),
        pltpu.VMEM((S, M), BF16),
        pltpu.VMEM((BQ, M), F32),
        pltpu.VMEM((M, 128), F32),
        pltpu.VMEM((6, 8, M), F32),
        pltpu.SemaphoreType.DMA((4 * NG,)),
        pltpu.SemaphoreType.DMA((2,)),
        pltpu.SemaphoreType.DMA((NG,)),
        pltpu.SemaphoreType.DMA((M // 128,)),
        pltpu.SemaphoreType.DMA((5,)),
        pltpu.SemaphoreType.DMA((S // BQ,)),
        pltpu.SemaphoreType.DMA((TOPK,)),
    ]
    out = pl.pallas_call(
        _kernel,
        in_specs=[hbm, hbm, hbm, hbm, hbm, hbm, vmem, hbm, hbm, hbm, vmem, hbm],
        out_specs=hbm,
        out_shape=jax.ShapeDtypeStruct((S, M), A_x.dtype),
        scratch_shapes=scratch,
        compiler_params=pltpu.CompilerParams(vmem_limit_bytes=124 * 1024 * 1024),
        name="adaln_cla_moe",
    )(A_x.reshape(S, M), A_c_kv.reshape(S, DC), A_w_q, A_w_uk, A_w_uv,
      A_w_o.reshape(H * D, M), B_w_r, B_w_gate.T, B_w_up.T, B_w_down, c, w_mod)
    return out.reshape(A_x.shape)
```

```python
import functools
import math

import jax
import jax.numpy as jnp
from jax import lax
import jax.experimental.pallas as pl
import jax.experimental.pallas.tpu as pltpu

F32 = jnp.float32
BF16 = jnp.bfloat16
U32 = jnp.uint32
I32 = jnp.int32

TOPK = 8
EPS = 1e-05
LOG2E = math.log2(math.e)
MASK_LOG2 = -1000000000.0 * LOG2E
BQ = 128
N_MXU = 4
HG = 8
A_STEPS = 4
HEADS_PER_ITER = 2
SUB_C = 2
LN_ROWS = 16
ST_ROWS = 16
LN1_GAP = 2
LN2_GAP = 3
END_GAP = 2
EXP_ROWS = 16
NT = (((1,), (1,)), ((), ()))


def _r(x):
    return x.astype(BF16).astype(F32)


def _dot(a, b):
    return jnp.dot(a, b, preferred_element_type=F32)


def _dot_nt(a, b):
    return lax.dot_general(a, b, NT, preferred_element_type=F32)


def _pack(x):
    return pltpu.bitcast(x.astype(BF16), U32)


def _unpack(x):
    return pltpu.bitcast(x, BF16)


def _ds(start, size):
    if not isinstance(start, int):
        start = pl.multiple_of(start, size)
    return pl.ds(start, size)


class _Pacer:
    def __init__(self):
        self.word = None

    def tick(self, x, gap=1):
        x = pltpu.bitcast(x, U32)
        tiles = [x[r:r + 8, c:c + 128]
                 for r in range(0, x.shape[0], 8) for c in range(0, x.shape[1], 128)]
        word = functools.reduce(jnp.bitwise_or, tiles)
        self.word = word if self.word is None else self.word | word
        self.idle(gap)

    def idle(self, gap):
        for _ in range(gap):
            self.word = pltpu.roll(self.word, 1, 1)


def _modulated_ln(x, shift, scale1):
    inv_n = 1.0 / x.shape[-1]
    mean = jnp.sum(x, axis=-1, keepdims=True) * inv_n
    xc = x - mean
    var = jnp.sum(xc * xc, axis=-1, keepdims=True) * inv_n
    std = _r(jnp.sqrt(_r(_r(var) + EPS)))
    n = _r(_r(x - _r(mean)) / std)
    return _r(_r(n * scale1) + shift)


def _attention(h0, h_v, wq_v, kv_v, vsum_v, ctx_v):
    H, B2, D = ctx_v.shape[0], BQ // 2, ctx_v.shape[2]
    S = 2 * ctx_v.shape[1]
    NB = S // BQ
    causal = (lax.broadcasted_iota(I32, (BQ, BQ), 1)
              <= lax.broadcasted_iota(I32, (BQ, BQ), 0))
    v_tail = {}
    for u in range(HEADS_PER_ITER):
        tot = None
        for i in range(NB - 1, 0, -1):
            part = vsum_v[h0 + u, i * 8:(i + 1) * 8, :]
            tot = part if tot is None else tot + part
            v_tail[u, i - 1] = tot

    steps = [(u, i) for u in range(HEADS_PER_ITER) for i in range(NB)]
    plan = [("q", *steps[0]), ("q", *steps[1]), ("s", *steps[0])]
    for t, step in enumerate(steps):
        plan += [("q", *st) for st in steps[t + 2:t + 3]]
        plan += [("s", *st) for st in steps[t + 1:t + 2]]
        plan.append(("o", *step))

    qs, scores = {}, {}
    tiles = 0
    inv = None
    for op, u, i in plan:
        h = h0 + u
        kend = (i + 1) * BQ
        if op == "q":
            q = _dot(_unpack(h_v[i * B2:(i + 1) * B2, :]), _unpack(wq_v[h]))
            qs[u, i] = (q * (D ** (-0.5) * LOG2E)).astype(BF16)
            tiles += h_v.shape[1] // 128
            continue
        if op == "s":
            s = _dot_nt(qs[u, i], _unpack(kv_v[h, :kend // 2, :]))
            sd = jnp.where(causal, s[:, kend - BQ:], MASK_LOG2)
            s = jnp.concatenate([s[:, :kend - BQ], sd], axis=1) if i else sd
            m = functools.reduce(jnp.maximum,
                                 [s[:, c:c + 128] for c in range(0, kend, 128)])
            if kend < S:
                m = jnp.concatenate([m[:-8], jnp.maximum(m[-8:], MASK_LOG2)], axis=0)
            scores[u, i] = s, jnp.max(m, axis=1, keepdims=True)
            tiles += i + 1
            continue
        s, m = scores[u, i]
        if inv is not None:
            m = jnp.where(inv < 0.0, inv, m)
        mb = jnp.broadcast_to(m, (BQ, 128))
        ps, ls, last = [], [None] * (BQ // EXP_ROWS), None
        lo, hi = 0, min(kend, (N_MXU - tiles % N_MXU) * BQ)
        while lo < kend:
            rows = []
            for e in range(BQ // EXP_ROWS):
                r = slice(e * EXP_ROWS, (e + 1) * EXP_ROWS)
                me = mb[r] if last is None else jnp.where(last < 0.0, last, mb[r])
                p = [jnp.exp2(s[r, c:c + 128] - me) for c in range(lo, hi, 128)]
                ls[e] = last = functools.reduce(
                    jnp.add, p if ls[e] is None else [ls[e]] + p)
                rows.append(jnp.concatenate(p, axis=1).astype(BF16))
            ps.append(jnp.concatenate(rows, axis=0))
            lo, hi = hi, min(kend, hi + N_MXU * BQ)
        l = jnp.sum(jnp.concatenate(ls, axis=0), axis=1, keepdims=True)
        o = _dot(jnp.concatenate(ps, axis=1), _unpack(kv_v[H + h, :kend // 2, :]))
        tiles += i + 1
        if kend < S:
            pm = jnp.exp2(MASK_LOG2 - m)
            l = l + pm * float(S - kend)
            o = o + pm * jnp.sum(v_tail[u, i], axis=0, keepdims=True)
        inv = pltpu.reciprocal(l, full_range=False)
        ctx_v[h, i * B2:(i + 1) * B2, :] = _pack(o * inv)


def _kernel(x_hbm, ckv_hbm, wq_hbm, wuk_hbm, wuv_hbm, wo_hbm, wr_ref, wgt_hbm,
            wut_hbm, wd_hbm, c_ref, wmod_hbm, out_hbm,
            x_v, ckv_v, wq_raw, wkv_raw, wo_v, wgt_v, wut_v, wd_v, wmod_v,
            a_v, h_v, wq_v, vsum_v, kv_v, ctx_v, x1_v, h2_v, out_v, pend_v, scol_v, mod_v,
            sem_kv, sem_ckv, sem_q, sem_mod, sem_in, sem_out, sem_fix):
    S, M = x_v.shape
    DC = ckv_v.shape[1]
    H, _, D = ctx_v.shape
    NG = H // HG
    NB = S // BQ
    B2 = BQ // 2
    NA = 4 * NG
    NM = M // 128
    NL = NA // 2
    N0 = NA - NL - NM
    MOD0 = 4

    def kv_copy(n):
        g, rows = n // 2, pl.ds((n % 2) * (DC // 2), DC // 2)
        src = wuk_hbm if g < NG else wuv_hbm
        return pltpu.make_async_copy(src.at[rows, pl.ds((g % NG) * HG, HG), :],
                                     wkv_raw.at[g, rows], sem_kv.at[n])

    def q_copy(g):
        return pltpu.make_async_copy(wq_hbm.at[:, pl.ds(g * HG, HG), :], wq_raw.at[g],
                                     sem_q.at[g])

    def row_copy(src, dst, sems, n, j):
        rows = pl.ds(j * n, n)
        return pltpu.make_async_copy(src.at[rows], dst.at[rows], sems.at[j])

    ckv_copy = functools.partial(row_copy, ckv_hbm, ckv_v, sem_ckv, S // 2)
    mod_copy = functools.partial(row_copy, wmod_hbm, wmod_v, sem_mod, 128)
    cp_x = pltpu.make_async_copy(x_hbm, x_v, sem_in.at[0])
    cp_wo = pltpu.make_async_copy(wo_hbm, wo_v, sem_in.at[1])
    cp_wg = pltpu.make_async_copy(wgt_hbm, wgt_v, sem_in.at[2])
    cp_wu = pltpu.make_async_copy(wut_hbm, wut_v, sem_in.at[3])
    cp_wd = pltpu.make_async_copy(wd_hbm, wd_v, sem_in.at[4])

    needs = []
    for n in range(NA):
        cps = [ckv_copy(n)] if n < 2 else []
        if n + 2 < NA:
            cps.append(kv_copy(n + 2))
        if N0 <= n < N0 + NM:
            cps.append(mod_copy(n - N0))
        if n == N0:
            cps += [q_copy(g) for g in range(NG)]
        if n == N0 + NM:
            cps.append(cp_x)
        needs.append(cps)

    needs += [[cp_wo], [cp_wg, cp_wu, cp_wd]]
    kv_copy(0).start()
    kv_copy(1).start()
    for cp in needs[0]:
        cp.start()

    cf = c_ref[...].astype(F32)
    scol_v[...] = jnp.broadcast_to(_r(cf * jax.nn.sigmoid(cf)), (128, M)).T
    pend_v[...] = jnp.zeros(pend_v.shape, F32)

    def stage_kv(n, lo, rows):
        src = jnp.minimum(n, NA - 1)
        w = wkv_raw[src // 2, _ds((src % 2) * (DC // 2) + lo, rows)]
        w = _pack(w.reshape(rows, HG * D))
        a_v[n % 4, lo // 2:(lo + rows) // 2, :] = w
        return w

    for n in range(2):
        kv_copy(n).wait()
        stage_kv(n, 0, DC // 2)

    def kv_loop(lo, hi, side_job):
        rows = S // 2 // A_STEPS

        def body(n, carry):
            for k in range(lo, hi):
                @pl.when(n == k)
                def _(k=k):
                    for cp in needs[k]:
                        cp.wait()
                    for cp in (needs[1] if k == 0 else []) + needs[k + 2]:
                        cp.start()

            g, half = n // 2, n % 2
            for st in range(A_STEPS):
                r0 = half * (S // 2) + st * rows
                w = jnp.concatenate([a_v[2 * (g % 2)], a_v[2 * (g % 2) + 1]], axis=0)
                kv = _dot(ckv_v[_ds(r0, rows), :], _unpack(w))
                if lo >= NA // 2:
                    for b in range(rows // BQ):
                        tot = functools.reduce(
                            jnp.add, [kv[e:e + 8] for e in range(b * BQ, (b + 1) * BQ, 8)])
                        for j in range(HG):
                            vsum_v[g * HG + j - H, _ds((r0 // BQ + b) * 8, 8), :] = (
                                tot[:, j * D:(j + 1) * D])
                kv = _pack(kv)
                for j in range(HG):
                    kv_v[g * HG + j, _ds(r0 // 2, rows // 2), :] = kv[:, j * D:(j + 1) * D]
            pacer = _Pacer()
            for r in range(0, DC // 2, ST_ROWS):
                pacer.tick(stage_kv(n + 2, r, ST_ROWS))
            side_job(n - lo, pacer)
            pacer.idle(END_GAP)
            a_v[MOD0, 64:72, 0:128] = pacer.word
            return carry

        lax.fori_loop(lo, hi, body, 0)

    def mod_and_wq(t, pacer):
        rows = _ds(t * 128, 128)
        tiles = [(i, j) for i in range(6) for j in range(M // 128)]
        for g in range(NG):
            for r in range(0, 128, ST_ROWS):
                if tiles:
                    i, j = tiles.pop(0)
                    prod = wmod_v[rows, i * M + j * 128:i * M + (j + 1) * 128].astype(F32)
                    prod = prod * scol_v[rows, :]
                    acc = functools.reduce(jnp.add, [prod[e:e + 8] for e in range(0, 128, 8)])
                    a_v[MOD0 + t, i * 8:(i + 1) * 8, j * 128:(j + 1) * 128] = (
                        pltpu.bitcast(acc, U32))
                    pacer.tick(acc, 0)
                w = _pack(wq_raw[g, _ds(t * 128 + r, ST_ROWS)].reshape(ST_ROWS, HG * D))
                for j in range(HG):
                    wq_v[g * HG + j, _ds(t * 64 + r // 2, ST_ROWS // 2), :] = (
                        w[:, j * D:(j + 1) * D])
                pacer.tick(w)
        assert not tiles

    def mod_row(i):
        return mod_v[i, 0:1, :]

    def ln1(t, pacer):
        for e in range(S // NL // LN_ROWS):
            r0 = t * (S // NL) + e * LN_ROWS
            xf = x_v[_ds(r0, LN_ROWS), :].astype(F32)
            h = _pack(_modulated_ln(xf, mod_row(0), mod_row(1)))
            h_v[_ds(r0 // 2, LN_ROWS // 2), :] = h
            pacer.tick(h, LN1_GAP)

    kv_loop(0, N0, lambda t, pacer: None)
    kv_loop(N0, N0 + NM, mod_and_wq)
    for i in range(6):
        parts = [pltpu.bitcast(a_v[MOD0 + t, i * 8:(i + 1) * 8, :M], F32)
                 for t in range(NM)]
        mod = _r(jnp.sum(functools.reduce(jnp.add, parts), axis=0, keepdims=True))
        if i % 3 == 1:
            mod = _r(1.0 + mod)
        mod_v[i] = jnp.broadcast_to(mod, (8, M))
    kv_loop(N0 + NM, NA, ln1)

    def heads_body(it, carry):
        _attention(it * HEADS_PER_ITER, h_v, wq_v, kv_v, vsum_v, ctx_v)
        return carry

    lax.fori_loop(0, H // HEADS_PER_ITER, heads_body, 0)

    cp_wo.wait()
    wr = wr_ref[...].astype(F32).reshape(1, M)

    def out_copy(blk):
        return pltpu.make_async_copy(out_v.at[_ds(blk * BQ, BQ), :],
                                     out_hbm.at[_ds(blk * BQ, BQ), :], sem_out.at[blk])

    def finish_rows(attn, r0, scores):
        n = attn.shape[0]
        rows = _ds(r0, n)
        x1 = _r(x_v[rows, :].astype(F32) + _r(mod_row(2) * _r(attn)))
        h2 = _modulated_ln(x1, mod_row(3), mod_row(4))
        out = x1 + _r(mod_row(5) * (h2 + h2 * 0.0))
        x1_v[rows, :] = x1.astype(BF16)
        h2_v[rows, :] = h2.astype(BF16)
        out = out.astype(BF16)
        out_v[rows, :] = out
        r = jnp.sum(h2 * wr, axis=1, keepdims=True)
        lane = lax.broadcasted_iota(I32, scores.shape, 1)
        for g in range(n // 8):
            scores = jnp.where(lane == r0 // 8 + g, r[g * 8:(g + 1) * 8], scores)
        return scores, out

    def c_body(t, scores):
        prev_blk = jnp.maximum(t * SUB_C - 1, 0)
        attn = pend_v[...]
        pacer = _Pacer()
        for b in range(SUB_C):
            blk = t * SUB_C + b
            for lo in range(0, BQ, LN_ROWS):
                scores, out = finish_rows(attn[lo:lo + LN_ROWS], prev_blk * BQ + lo, scores)
                pacer.tick(scores, 0)
                pacer.tick(out, LN2_GAP)
            ctx = jnp.concatenate([ctx_v[h, _ds(blk * B2, B2), :] for h in range(H)], axis=1)
            attn = _dot(_unpack(ctx), wo_v[...])
            prev_blk = blk
        pend_v[...] = attn
        a_v[MOD0, 64:72, 0:128] = pacer.word

        @pl.when(t > 0)
        def _():
            out_copy(t * SUB_C - 1).start()

        for b in range(SUB_C - 1):
            out_copy(t * SUB_C + b).start()
        return scores

    scores = jnp.zeros((8, S // 8), F32)
    scores = lax.fori_loop(0, NB // SUB_C, c_body, scores)
    scores, _ = finish_rows(pend_v[...], (NB - 1) * BQ, scores)
    out_copy(NB - 1).start()

    rb = _r(scores)
    bits = pltpu.bitcast(jnp.where(rb == 0.0, 0.0, rb), I32)
    k16 = (bits >> 16) & 0xFFFF
    k16 = jnp.where(bits < 0, 0xFFFF - k16, k16 + 0x8000)
    k16 = jnp.where(rb != rb, 0, k16)
    ridx = (lax.broadcasted_iota(I32, scores.shape, 1) * 8
            + lax.broadcasted_iota(I32, scores.shape, 0))
    idx_bits = (S - 1).bit_length()
    key = pltpu.bitcast((k16 << idx_bits) + (S - 1 - ridx) + (1 << 29), F32)
    picks = []
    for _ in range(TOPK):
        top = jnp.max(jnp.max(key, axis=1, keepdims=True), axis=0, keepdims=True)
        key = jnp.where(key == top, 1.0e-30, key)
        picks.append(S - 1 - (pltpu.bitcast(top, I32)[0, 0] & ((1 << idx_bits) - 1)))

    row16 = lax.broadcasted_iota(I32, (16, M), 0)

    def tile_of(i):
        return _ds((i // 16) * 16, 16)

    sel = jnp.zeros((16, M), F32)
    for j, i in enumerate(picks):
        tile = h2_v[tile_of(i), :].astype(F32)
        hrow = jnp.sum(jnp.where(row16 == i % 16, tile, 0.0), axis=0, keepdims=True)
        sel = jnp.where(row16 == j, hrow, sel)

    cp_wg.wait()
    cp_wu.wait()
    cp_wd.wait()
    sel_b = sel.astype(BF16)
    g = _r(_dot_nt(sel_b, wgt_v[...]))
    g = _r(g * jax.nn.sigmoid(g))
    u = _r(_dot_nt(sel_b, wut_v[...]))
    y = _r(_dot((g * u).astype(BF16), wd_v[...]))
    gate = _r(jax.nn.sigmoid(_r(jnp.sum(sel * wr, axis=1, keepdims=True))))
    y = _r(y * gate)
    delta = _r(mod_row(5) * _r(sel + _r(sel * 0.0 + y)))

    for t in range(NB):
        out_copy(t).wait()
    for j, i in enumerate(picks):
        new = (x1_v[tile_of(i), :].astype(F32) + delta[j:j + 1, :]).astype(BF16)
        out_v[tile_of(i), :] = jnp.where(row16 == i % 16, new, out_v[tile_of(i), :])

    def fix_copy(j):
        return pltpu.make_async_copy(out_v.at[tile_of(picks[j]), :],
                                     out_hbm.at[tile_of(picks[j]), :], sem_fix.at[j])

    first = []
    for j in range(TOPK):
        f = jnp.bool_(True)
        for e in range(j):
            f = jnp.logical_and(f, picks[e] // 16 != picks[j] // 16)
        first.append(f)
    for j in range(TOPK):
        pl.when(first[j])(fix_copy(j).start)
    for j in range(TOPK):
        pl.when(first[j])(fix_copy(j).wait)


@jax.jit
def pallas_adaLN_cond__compressed_kv_cla__moe_arch_mod__prompt_kernel(
    A_x: jax.Array,
    A_c_kv: jax.Array,
    A_w_q: jax.Array,
    A_w_uk: jax.Array,
    A_w_uv: jax.Array,
    A_w_o: jax.Array,
    B_x: jax.Array,
    B_w_r: jax.Array,
    B_w_gate: jax.Array,
    B_w_up: jax.Array,
    B_w_down: jax.Array,
    c: jax.Array,
    w_mod: jax.Array,
):
    del B_x
    _, S, M = A_x.shape
    DC = A_c_kv.shape[2]
    _, H, D = A_w_q.shape
    F = B_w_gate.shape[1]
    NG = H // HG

    hbm = pl.BlockSpec(memory_space=pl.ANY)
    vmem = pl.BlockSpec(memory_space=pltpu.VMEM)
    scratch = [
        pltpu.VMEM((S, M), BF16),
        pltpu.VMEM((S, DC), BF16),
        pltpu.VMEM((NG, M, HG, D), BF16),
        pltpu.VMEM((2 * NG, DC, HG, D), BF16),
        pltpu.VMEM((H * D, M), BF16),
        pltpu.VMEM((F, M), BF16),
        pltpu.VMEM((F, M), BF16),
        pltpu.VMEM((F, M), BF16),
        pltpu.VMEM((M, 6 * M), BF16),
        pltpu.VMEM((4 + M // 128, DC // 4, HG * D), U32),
        pltpu.VMEM((S // 2, M), U32),
        pltpu.VMEM((H, M // 2, D), U32),
        pltpu.VMEM((H, S // BQ * 8, D), F32),
        pltpu.VMEM((2 * H, S // 2, D), U32),
        pltpu.VMEM((H, S // 2, D), U32),
        pltpu.VMEM((S, M), BF16),
        pltpu.VMEM((S, M), BF16),
        pltpu.VMEM((S, M), BF16),
        pltpu.VMEM((BQ, M), F32),
        pltpu.VMEM((M, 128), F32),
        pltpu.VMEM((6, 8, M), F32),
        pltpu.SemaphoreType.DMA((4 * NG,)),
        pltpu.SemaphoreType.DMA((2,)),
        pltpu.SemaphoreType.DMA((NG,)),
        pltpu.SemaphoreType.DMA((M // 128,)),
        pltpu.SemaphoreType.DMA((5,)),
        pltpu.SemaphoreType.DMA((S // BQ,)),
        pltpu.SemaphoreType.DMA((TOPK,)),
    ]
    out = pl.pallas_call(
        _kernel,
        in_specs=[hbm, hbm, hbm, hbm, hbm, hbm, vmem, hbm, hbm, hbm, vmem, hbm],
        out_specs=hbm,
        out_shape=jax.ShapeDtypeStruct((S, M), A_x.dtype),
        scratch_shapes=scratch,
        compiler_params=pltpu.CompilerParams(vmem_limit_bytes=124 * 1024 * 1024),
        name="adaln_cla_moe",
    )(A_x.reshape(S, M), A_c_kv.reshape(S, DC), A_w_q, A_w_uk, A_w_uv,
      A_w_o.reshape(H * D, M), B_w_r, B_w_gate.T, B_w_up.T, B_w_down, c, w_mod)
    return out.reshape(A_x.shape)
```

```python
import functools
import math

import jax
import jax.numpy as jnp
from jax import lax
import jax.experimental.pallas as pl
import jax.experimental.pallas.tpu as pltpu

F32 = jnp.float32
BF16 = jnp.bfloat16
U32 = jnp.uint32
I32 = jnp.int32

TOPK = 8
EPS = 1e-05
LOG2E = math.log2(math.e)
MASK_LOG2 = -1000000000.0 * LOG2E
BQ = 128
N_MXU = 4
HG = 8
A_STEPS = 4
HEADS_PER_ITER = 2
SUB_C = 2
LN_ROWS = 16
ST_ROWS = 16
LN1_GAP = 2
LN2_GAP = 3
END_GAP = 2
EXP_ROWS = 16
NT = (((1,), (1,)), ((), ()))


def _r(x):
    return x.astype(BF16).astype(F32)


def _dot(a, b):
    return jnp.dot(a, b, preferred_element_type=F32)


def _dot_nt(a, b):
    return lax.dot_general(a, b, NT, preferred_element_type=F32)


def _pack(x):
    return pltpu.bitcast(x.astype(BF16), U32)


def _unpack(x):
    return pltpu.bitcast(x, BF16)


def _ds(start, size):
    if not isinstance(start, int):
        start = pl.multiple_of(start, size)
    return pl.ds(start, size)


class _Pacer:
    def __init__(self):
        self.word = None

    def tick(self, x, gap=1):
        x = pltpu.bitcast(x, U32)
        tiles = [x[r:r + 8, c:c + 128]
                 for r in range(0, x.shape[0], 8) for c in range(0, x.shape[1], 128)]
        word = functools.reduce(jnp.bitwise_or, tiles)
        self.word = word if self.word is None else self.word | word
        self.idle(gap)

    def idle(self, gap):
        for _ in range(gap):
            self.word = pltpu.roll(self.word, 1, 1)


def _modulated_ln(x, shift, scale1):
    inv_n = 1.0 / x.shape[-1]
    mean = jnp.sum(x, axis=-1, keepdims=True) * inv_n
    xc = x - mean
    var = jnp.sum(xc * xc, axis=-1, keepdims=True) * inv_n
    std = _r(jnp.sqrt(_r(_r(var) + EPS)))
    n = _r(_r(x - _r(mean)) / std)
    return _r(_r(n * scale1) + shift)


def _attention(h0, h_v, wq_v, kv_v, vsum_v, ctx_v):
    H, B2, D = ctx_v.shape[0], BQ // 2, ctx_v.shape[2]
    S = 2 * ctx_v.shape[1]
    NB = S // BQ
    causal = (lax.broadcasted_iota(I32, (BQ, BQ), 1)
              <= lax.broadcasted_iota(I32, (BQ, BQ), 0))
    v_tail = {}
    for u in range(HEADS_PER_ITER):
        tot = None
        for i in range(NB - 1, 0, -1):
            part = vsum_v[h0 + u, i * 8:(i + 1) * 8, :]
            tot = part if tot is None else tot + part
            v_tail[u, i - 1] = tot

    steps = [(u, i) for u in range(HEADS_PER_ITER) for i in range(NB)]
    plan = [("q", *steps[0]), ("q", *steps[1]), ("s", *steps[0])]
    for t, step in enumerate(steps):
        plan += [("q", *st) for st in steps[t + 2:t + 3]]
        plan += [("s", *st) for st in steps[t + 1:t + 2]]
        plan.append(("o", *step))

    qs, scores = {}, {}
    tiles = 0
    inv = None
    for op, u, i in plan:
        h = h0 + u
        kend = (i + 1) * BQ
        if op == "q":
            q = _dot(_unpack(h_v[i * B2:(i + 1) * B2, :]), _unpack(wq_v[h]))
            qs[u, i] = (q * (D ** (-0.5) * LOG2E)).astype(BF16)
            tiles += h_v.shape[1] // 128
            continue
        if op == "s":
            s = _dot_nt(qs[u, i], _unpack(kv_v[h, :kend // 2, :]))
            sd = jnp.where(causal, s[:, kend - BQ:], MASK_LOG2)
            s = jnp.concatenate([s[:, :kend - BQ], sd], axis=1) if i else sd
            m = functools.reduce(jnp.maximum,
                                 [s[:, c:c + 128] for c in range(0, kend, 128)])
            if kend < S:
                m = jnp.concatenate([m[:-8], jnp.maximum(m[-8:], MASK_LOG2)], axis=0)
            scores[u, i] = s, jnp.max(m, axis=1, keepdims=True)
            tiles += i + 1
            continue
        s, m = scores[u, i]
        if inv is not None:
            m = jnp.where(inv < 0.0, inv, m)
        mb = jnp.broadcast_to(m, (BQ, 128))
        ps, ls, last = [], [None] * (BQ // EXP_ROWS), None
        lo, hi = 0, min(kend, (N_MXU - tiles % N_MXU) * BQ)
        while lo < kend:
            rows = []
            for e in range(BQ // EXP_ROWS):
                r = slice(e * EXP_ROWS, (e + 1) * EXP_ROWS)
                me = mb[r] if last is None else jnp.where(last < 0.0, last, mb[r])
                p = [jnp.exp2(s[r, c:c + 128] - me) for c in range(lo, hi, 128)]
                ls[e] = last = functools.reduce(
                    jnp.add, p if ls[e] is None else [ls[e]] + p)
                rows.append(jnp.concatenate(p, axis=1).astype(BF16))
            ps.append(jnp.concatenate(rows, axis=0))
            lo, hi = hi, min(kend, hi + N_MXU * BQ)
        l = jnp.sum(jnp.concatenate(ls, axis=0), axis=1, keepdims=True)
        o = _dot(jnp.concatenate(ps, axis=1), _unpack(kv_v[H + h, :kend // 2, :]))
        tiles += i + 1
        if kend < S:
            pm = jnp.exp2(MASK_LOG2 - m)
            l = l + pm * float(S - kend)
            o = o + pm * jnp.sum(v_tail[u, i], axis=0, keepdims=True)
        inv = pltpu.reciprocal(l, full_range=False)
        ctx_v[h, i * B2:(i + 1) * B2, :] = _pack(o * inv)


def _kernel(x_hbm, ckv_hbm, wq_hbm, wuk_hbm, wuv_hbm, wo_hbm, wr_hbm, wgt_hbm,
            wut_hbm, wd_hbm, c_hbm, wmod_hbm, out_hbm,
            x_v, ckv_v, wq_raw, wkv_raw, wo_v, wgt_v, wut_v, wd_v, wmod_v,
            a_v, h_v, wq_v, vsum_v, kv_v, ctx_v, x1_v, h2_v, out_v, pend_v, scol_v, mod_v,
            c_v, wr_v,
            sem_kv, sem_ckv, sem_q, sem_mod, sem_in, sem_out, sem_fix):
    S, M = x_v.shape
    DC = ckv_v.shape[1]
    H, _, D = ctx_v.shape
    NG = H // HG
    NB = S // BQ
    B2 = BQ // 2
    NA = 4 * NG
    NM = M // 128
    NL = NA // 2
    N0 = NA - NL - NM
    MOD0 = 4

    def kv_copy(n):
        g, rows = n // 2, pl.ds((n % 2) * (DC // 2), DC // 2)
        src = wuk_hbm if g < NG else wuv_hbm
        return pltpu.make_async_copy(src.at[rows, pl.ds((g % NG) * HG, HG), :],
                                     wkv_raw.at[g, rows], sem_kv.at[n])

    def q_copy(g):
        return pltpu.make_async_copy(wq_hbm.at[:, pl.ds(g * HG, HG), :], wq_raw.at[g],
                                     sem_q.at[g])

    def row_copy(src, dst, sems, n, j):
        rows = pl.ds(j * n, n)
        return pltpu.make_async_copy(src.at[rows], dst.at[rows], sems.at[j])

    ckv_copy = functools.partial(row_copy, ckv_hbm, ckv_v, sem_ckv, S // 2)
    mod_copy = functools.partial(row_copy, wmod_hbm, wmod_v, sem_mod, 128)
    cp_x = pltpu.make_async_copy(x_hbm, x_v, sem_in.at[0])
    cp_wo = pltpu.make_async_copy(wo_hbm, wo_v, sem_in.at[1])
    cp_wg = pltpu.make_async_copy(wgt_hbm, wgt_v, sem_in.at[2])
    cp_wu = pltpu.make_async_copy(wut_hbm, wut_v, sem_in.at[3])
    cp_wd = pltpu.make_async_copy(wd_hbm, wd_v, sem_in.at[4])
    cp_wr = pltpu.make_async_copy(wr_hbm, wr_v, sem_in.at[5])
    cp_c = pltpu.make_async_copy(c_hbm, c_v, sem_in.at[6])

    needs = []
    for n in range(NA):
        cps = [ckv_copy(n)] if n < 2 else []
        if n == 1:
            cps.append(kv_copy(2))
        if n and n + 2 < NA:
            cps.append(kv_copy(n + 2))
        if N0 <= n < N0 + NM:
            cps.append(mod_copy(n - N0))
        if n == N0:
            cps += [q_copy(g) for g in range(NG)]
        if n == N0 + NM:
            cps.append(cp_x)
        needs.append(cps)

    needs += [[cp_wo, cp_wr], [cp_wg, cp_wu, cp_wd]]
    cp_c.start()
    kv_copy(0).start()
    kv_copy(1).start()
    for cp in needs[0]:
        cp.start()

    pend_v[...] = jnp.zeros(pend_v.shape, F32)
    cp_c.wait()
    cf = c_v[...].astype(F32)
    scol_v[...] = jnp.broadcast_to(_r(cf * jax.nn.sigmoid(cf)), (128, M)).T

    def stage_kv(src, slab, lo, rows):
        w = wkv_raw[src // 2, _ds((src % 2) * (DC // 2) + lo, rows)]
        w = _pack(w.reshape(rows, HG * D))
        a_v[slab, lo // 2:(lo + rows) // 2, :] = w
        return w

    for n in range(2):
        kv_copy(n).wait()
        stage_kv(n, n, 0, DC // 2)

    def kv_loop(lo, hi, side_job):
        rows = S // 2 // A_STEPS

        def body(n, carry):
            for k in range(lo, hi):
                @pl.when(n == k)
                def _(k=k):
                    for cp in needs[k]:
                        cp.wait()
                    for cp in (needs[1] if k == 0 else []) + needs[k + 2]:
                        cp.start()

            g, half = n // 2, n % 2
            for st in range(A_STEPS):
                r0 = half * (S // 2) + st * rows
                w = jnp.concatenate([a_v[2 * (g % 2)], a_v[2 * (g % 2) + 1]], axis=0)
                kv = _dot(ckv_v[_ds(r0, rows), :], _unpack(w))
                if lo >= NA // 2:
                    for b in range(rows // BQ):
                        tot = functools.reduce(
                            jnp.add, [kv[e:e + 8] for e in range(b * BQ, (b + 1) * BQ, 8)])
                        for j in range(HG):
                            vsum_v[g * HG + j - H, _ds((r0 // BQ + b) * 8, 8), :] = (
                                tot[:, j * D:(j + 1) * D])
                kv = _pack(kv)
                for j in range(HG):
                    kv_v[g * HG + j, _ds(r0 // 2, rows // 2), :] = kv[:, j * D:(j + 1) * D]
            pacer = _Pacer()
            src = jnp.where(n == 0, 0, jnp.minimum(n + 2, NA - 1))
            for r in range(0, DC // 2, ST_ROWS):
                pacer.tick(stage_kv(src, (n + 2) % 4, r, ST_ROWS))
            side_job(n - lo, pacer)
            pacer.idle(END_GAP)
            a_v[MOD0, 64:72, 0:128] = pacer.word
            return carry

        lax.fori_loop(lo, hi, body, 0)

    def mod_and_wq(t, pacer):
        rows = _ds(t * 128, 128)
        tiles = [(i, j) for i in range(6) for j in range(M // 128)]
        for g in range(NG):
            for r in range(0, 128, ST_ROWS):
                if tiles:
                    i, j = tiles.pop(0)
                    prod = wmod_v[rows, i * M + j * 128:i * M + (j + 1) * 128].astype(F32)
                    prod = prod * scol_v[rows, :]
                    acc = functools.reduce(jnp.add, [prod[e:e + 8] for e in range(0, 128, 8)])
                    a_v[MOD0 + t, i * 8:(i + 1) * 8, j * 128:(j + 1) * 128] = (
                        pltpu.bitcast(acc, U32))
                    pacer.tick(acc, 0)
                w = _pack(wq_raw[g, _ds(t * 128 + r, ST_ROWS)].reshape(ST_ROWS, HG * D))
                for j in range(HG):
                    wq_v[g * HG + j, _ds(t * 64 + r // 2, ST_ROWS // 2), :] = (
                        w[:, j * D:(j + 1) * D])
                pacer.tick(w)
        assert not tiles

    def mod_row(i):
        return mod_v[i, 0:1, :]

    def ln1(t, pacer):
        for e in range(S // NL // LN_ROWS):
            r0 = t * (S // NL) + e * LN_ROWS
            xf = x_v[_ds(r0, LN_ROWS), :].astype(F32)
            h = _pack(_modulated_ln(xf, mod_row(0), mod_row(1)))
            h_v[_ds(r0 // 2, LN_ROWS // 2), :] = h
            pacer.tick(h, LN1_GAP)

    def catch_up(t, pacer):
        for r in range(0, DC // 2, ST_ROWS):
            pacer.tick(stage_kv(jnp.where(t == 1, 2, 0), jnp.where(t == 1, 2, MOD0 + 1),
                                r, ST_ROWS))

    kv_loop(0, N0, catch_up)
    kv_loop(N0, N0 + NM, mod_and_wq)
    for i in range(6):
        parts = [pltpu.bitcast(a_v[MOD0 + t, i * 8:(i + 1) * 8, :M], F32)
                 for t in range(NM)]
        mod = _r(jnp.sum(functools.reduce(jnp.add, parts), axis=0, keepdims=True))
        if i % 3 == 1:
            mod = _r(1.0 + mod)
        mod_v[i] = jnp.broadcast_to(mod, (8, M))
    kv_loop(N0 + NM, NA, ln1)

    def heads_body(it, carry):
        _attention(it * HEADS_PER_ITER, h_v, wq_v, kv_v, vsum_v, ctx_v)
        return carry

    lax.fori_loop(0, H // HEADS_PER_ITER, heads_body, 0)

    cp_wo.wait()
    cp_wr.wait()
    wr = wr_v[...].astype(F32).reshape(1, M)

    def out_copy(blk):
        return pltpu.make_async_copy(out_v.at[_ds(blk * BQ, BQ), :],
                                     out_hbm.at[_ds(blk * BQ, BQ), :], sem_out.at[blk])

    def finish_rows(attn, r0, scores):
        n = attn.shape[0]
        rows = _ds(r0, n)
        x1 = _r(x_v[rows, :].astype(F32) + _r(mod_row(2) * _r(attn)))
        h2 = _modulated_ln(x1, mod_row(3), mod_row(4))
        out = x1 + _r(mod_row(5) * (h2 + h2 * 0.0))
        x1_v[rows, :] = x1.astype(BF16)
        h2_v[rows, :] = h2.astype(BF16)
        out = out.astype(BF16)
        out_v[rows, :] = out
        r = jnp.sum(h2 * wr, axis=1, keepdims=True)
        lane = lax.broadcasted_iota(I32, scores.shape, 1)
        for g in range(n // 8):
            scores = jnp.where(lane == r0 // 8 + g, r[g * 8:(g + 1) * 8], scores)
        return scores, out

    def c_body(t, scores):
        prev_blk = jnp.maximum(t * SUB_C - 1, 0)
        attn = pend_v[...]
        pacer = _Pacer()
        for b in range(SUB_C):
            blk = t * SUB_C + b
            for lo in range(0, BQ, LN_ROWS):
                scores, out = finish_rows(attn[lo:lo + LN_ROWS], prev_blk * BQ + lo, scores)
                pacer.tick(scores, 0)
                pacer.tick(out, LN2_GAP)
            ctx = jnp.concatenate([ctx_v[h, _ds(blk * B2, B2), :] for h in range(H)], axis=1)
            attn = _dot(_unpack(ctx), wo_v[...])
            prev_blk = blk
        pend_v[...] = attn
        a_v[MOD0, 64:72, 0:128] = pacer.word

        @pl.when(t > 0)
        def _():
            out_copy(t * SUB_C - 1).start()

        for b in range(SUB_C - 1):
            out_copy(t * SUB_C + b).start()
        return scores

    scores = jnp.zeros((8, S // 8), F32)
    scores = lax.fori_loop(0, NB // SUB_C, c_body, scores)
    scores, _ = finish_rows(pend_v[...], (NB - 1) * BQ, scores)
    out_copy(NB - 1).start()

    rb = _r(scores)
    bits = pltpu.bitcast(jnp.where(rb == 0.0, 0.0, rb), I32)
    k16 = (bits >> 16) & 0xFFFF
    k16 = jnp.where(bits < 0, 0xFFFF - k16, k16 + 0x8000)
    k16 = jnp.where(rb != rb, 0, k16)
    ridx = (lax.broadcasted_iota(I32, scores.shape, 1) * 8
            + lax.broadcasted_iota(I32, scores.shape, 0))
    idx_bits = (S - 1).bit_length()
    key = pltpu.bitcast((k16 << idx_bits) + (S - 1 - ridx) + (1 << 29), F32)
    picks = []
    for _ in range(TOPK):
        top = jnp.max(jnp.max(key, axis=1, keepdims=True), axis=0, keepdims=True)
        key = jnp.where(key == top, 1.0e-30, key)
        picks.append(S - 1 - (pltpu.bitcast(top, I32)[0, 0] & ((1 << idx_bits) - 1)))

    row16 = lax.broadcasted_iota(I32, (16, M), 0)

    def tile_of(i):
        return _ds((i // 16) * 16, 16)

    sel = jnp.zeros((16, M), F32)
    for j, i in enumerate(picks):
        tile = h2_v[tile_of(i), :].astype(F32)
        hrow = jnp.sum(jnp.where(row16 == i % 16, tile, 0.0), axis=0, keepdims=True)
        sel = jnp.where(row16 == j, hrow, sel)

    cp_wg.wait()
    cp_wu.wait()
    cp_wd.wait()
    sel_b = sel.astype(BF16)
    g = _r(_dot_nt(sel_b, wgt_v[...]))
    g = _r(g * jax.nn.sigmoid(g))
    u = _r(_dot_nt(sel_b, wut_v[...]))
    y = _r(_dot((g * u).astype(BF16), wd_v[...]))
    gate = _r(jax.nn.sigmoid(_r(jnp.sum(sel * wr, axis=1, keepdims=True))))
    y = _r(y * gate)
    delta = _r(mod_row(5) * _r(sel + _r(sel * 0.0 + y)))

    for t in range(NB):
        out_copy(t).wait()
    for j, i in enumerate(picks):
        new = (x1_v[tile_of(i), :].astype(F32) + delta[j:j + 1, :]).astype(BF16)
        out_v[tile_of(i), :] = jnp.where(row16 == i % 16, new, out_v[tile_of(i), :])

    def fix_copy(j):
        return pltpu.make_async_copy(out_v.at[tile_of(picks[j]), :],
                                     out_hbm.at[tile_of(picks[j]), :], sem_fix.at[j])

    first = []
    for j in range(TOPK):
        f = jnp.bool_(True)
        for e in range(j):
            f = jnp.logical_and(f, picks[e] // 16 != picks[j] // 16)
        first.append(f)
    for j in range(TOPK):
        pl.when(first[j])(fix_copy(j).start)
    for j in range(TOPK):
        pl.when(first[j])(fix_copy(j).wait)


@jax.jit
def pallas_adaLN_cond__compressed_kv_cla__moe_arch_mod__prompt_kernel(
    A_x: jax.Array,
    A_c_kv: jax.Array,
    A_w_q: jax.Array,
    A_w_uk: jax.Array,
    A_w_uv: jax.Array,
    A_w_o: jax.Array,
    B_x: jax.Array,
    B_w_r: jax.Array,
    B_w_gate: jax.Array,
    B_w_up: jax.Array,
    B_w_down: jax.Array,
    c: jax.Array,
    w_mod: jax.Array,
):
    del B_x
    _, S, M = A_x.shape
    DC = A_c_kv.shape[2]
    _, H, D = A_w_q.shape
    F = B_w_gate.shape[1]
    NG = H // HG

    hbm = pl.BlockSpec(memory_space=pl.ANY)
    scratch = [
        pltpu.VMEM((S, M), BF16),
        pltpu.VMEM((S, DC), BF16),
        pltpu.VMEM((NG, M, HG, D), BF16),
        pltpu.VMEM((2 * NG, DC, HG, D), BF16),
        pltpu.VMEM((H * D, M), BF16),
        pltpu.VMEM((F, M), BF16),
        pltpu.VMEM((F, M), BF16),
        pltpu.VMEM((F, M), BF16),
        pltpu.VMEM((M, 6 * M), BF16),
        pltpu.VMEM((4 + M // 128, DC // 4, HG * D), U32),
        pltpu.VMEM((S // 2, M), U32),
        pltpu.VMEM((H, M // 2, D), U32),
        pltpu.VMEM((H, S // BQ * 8, D), F32),
        pltpu.VMEM((2 * H, S // 2, D), U32),
        pltpu.VMEM((H, S // 2, D), U32),
        pltpu.VMEM((S, M), BF16),
        pltpu.VMEM((S, M), BF16),
        pltpu.VMEM((S, M), BF16),
        pltpu.VMEM((BQ, M), F32),
        pltpu.VMEM((M, 128), F32),
        pltpu.VMEM((6, 8, M), F32),
        pltpu.VMEM((1, M), BF16),
        pltpu.VMEM((M,), BF16),
        pltpu.SemaphoreType.DMA((4 * NG,)),
        pltpu.SemaphoreType.DMA((2,)),
        pltpu.SemaphoreType.DMA((NG,)),
        pltpu.SemaphoreType.DMA((M // 128,)),
        pltpu.SemaphoreType.DMA((7,)),
        pltpu.SemaphoreType.DMA((S // BQ,)),
        pltpu.SemaphoreType.DMA((TOPK,)),
    ]
    out = pl.pallas_call(
        _kernel,
        in_specs=[hbm] * 12,
        out_specs=hbm,
        out_shape=jax.ShapeDtypeStruct((S, M), A_x.dtype),
        scratch_shapes=scratch,
        compiler_params=pltpu.CompilerParams(vmem_limit_bytes=124 * 1024 * 1024),
        name="adaln_cla_moe",
    )(A_x.reshape(S, M), A_c_kv.reshape(S, DC), A_w_q, A_w_uk, A_w_uv,
      A_w_o.reshape(H * D, M), B_w_r, B_w_gate.T, B_w_up.T, B_w_down, c, w_mod)
    return out.reshape(A_x.shape)
```

```python
import functools
import math

import jax
import jax.numpy as jnp
from jax import lax
import jax.experimental.pallas as pl
import jax.experimental.pallas.tpu as pltpu

F32 = jnp.float32
BF16 = jnp.bfloat16
U32 = jnp.uint32
I32 = jnp.int32

TOPK = 8
EPS = 1e-05
LOG2E = math.log2(math.e)
MASK_LOG2 = -1000000000.0 * LOG2E
BQ = 128
N_MXU = 4
HG = 8
A_STEPS = 2
HEADS_PER_ITER = 2
SUB_C = 2
LN_ROWS = 16
ST_ROWS = 16
LN1_GAP = 2
LN2_GAP = 4
END_GAP = 2
EXP_ROWS = 16
NT = (((1,), (1,)), ((), ()))


def _r(x):
    return x.astype(BF16).astype(F32)


def _dot(a, b):
    return jnp.dot(a, b, preferred_element_type=F32)


def _dot_nt(a, b):
    return lax.dot_general(a, b, NT, preferred_element_type=F32)


def _pack(x):
    return pltpu.bitcast(x.astype(BF16), U32)


def _unpack(x):
    return pltpu.bitcast(x, BF16)


def _ds(start, size):
    if not isinstance(start, int):
        start = pl.multiple_of(start, size)
    return pl.ds(start, size)


class _Pacer:
    def __init__(self):
        self.word = None

    def tick(self, x, gap=1):
        x = pltpu.bitcast(x, U32)
        tiles = [x[r:r + 8, c:c + 128]
                 for r in range(0, x.shape[0], 8) for c in range(0, x.shape[1], 128)]
        word = functools.reduce(jnp.bitwise_or, tiles)
        self.word = word if self.word is None else self.word | word
        self.idle(gap)

    def idle(self, gap):
        for _ in range(gap):
            self.word = pltpu.roll(self.word, 1, 1)


def _modulated_ln(x, shift, scale1):
    inv_n = 1.0 / x.shape[-1]
    mean = jnp.sum(x, axis=-1, keepdims=True) * inv_n
    xc = x - mean
    var = jnp.sum(xc * xc, axis=-1, keepdims=True) * inv_n
    std = _r(jnp.sqrt(_r(_r(var) + EPS)))
    n = _r(_r(x - _r(mean)) / std)
    return _r(_r(n * scale1) + shift)


def _attention(h0, h_v, wq_v, kv_v, vsum_v, ctx_v):
    H, B2, D = ctx_v.shape[0], BQ // 2, ctx_v.shape[2]
    S = 2 * ctx_v.shape[1]
    NB = S // BQ
    causal = (lax.broadcasted_iota(I32, (BQ, BQ), 1)
              <= lax.broadcasted_iota(I32, (BQ, BQ), 0))
    v_tail = {}
    for u in range(HEADS_PER_ITER):
        tot = None
        for i in range(NB - 1, 0, -1):
            part = vsum_v[h0 + u, i * 8:(i + 1) * 8, :]
            tot = part if tot is None else tot + part
            v_tail[u, i - 1] = tot

    steps = [(u, i) for u in range(HEADS_PER_ITER) for i in range(NB)]
    plan = [("q", *steps[0]), ("q", *steps[1]), ("s", *steps[0])]
    for t, step in enumerate(steps):
        plan += [("q", *st) for st in steps[t + 2:t + 3]]
        plan += [("s", *st) for st in steps[t + 1:t + 2]]
        plan.append(("o", *step))

    qs, scores = {}, {}
    tiles = 0
    inv = None
    for op, u, i in plan:
        h = h0 + u
        kend = (i + 1) * BQ
        if op == "q":
            q = _dot(_unpack(h_v[i * B2:(i + 1) * B2, :]), _unpack(wq_v[h]))
            qs[u, i] = (q * (D ** (-0.5) * LOG2E)).astype(BF16)
            tiles += h_v.shape[1] // 128
            continue
        if op == "s":
            s = _dot_nt(qs[u, i], _unpack(kv_v[h, :kend // 2, :]))
            sd = jnp.where(causal, s[:, kend - BQ:], MASK_LOG2)
            s = jnp.concatenate([s[:, :kend - BQ], sd], axis=1) if i else sd
            m = functools.reduce(jnp.maximum,
                                 [s[:, c:c + 128] for c in range(0, kend, 128)])
            if kend < S:
                m = jnp.concatenate([m[:-8], jnp.maximum(m[-8:], MASK_LOG2)], axis=0)
            scores[u, i] = s, jnp.max(m, axis=1, keepdims=True)
            tiles += i + 1
            continue
        s, m = scores[u, i]
        if inv is not None:
            m = jnp.where(inv < 0.0, inv, m)
        mb = jnp.broadcast_to(m, (BQ, 128))
        ps, ls, last = [], [None] * (BQ // EXP_ROWS), None
        lo, hi = 0, min(kend, (N_MXU - tiles % N_MXU) * BQ)
        while lo < kend:
            rows = []
            for e in range(BQ // EXP_ROWS):
                r = slice(e * EXP_ROWS, (e + 1) * EXP_ROWS)
                me = mb[r] if last is None else jnp.where(last < 0.0, last, mb[r])
                p = [jnp.exp2(s[r, c:c + 128] - me) for c in range(lo, hi, 128)]
                ls[e] = last = functools.reduce(
                    jnp.add, p if ls[e] is None else [ls[e]] + p)
                rows.append(jnp.concatenate(p, axis=1).astype(BF16))
            ps.append(jnp.concatenate(rows, axis=0))
            lo, hi = hi, min(kend, hi + N_MXU * BQ)
        l = jnp.sum(jnp.concatenate(ls, axis=0), axis=1, keepdims=True)
        o = _dot(jnp.concatenate(ps, axis=1), _unpack(kv_v[H + h, :kend // 2, :]))
        tiles += i + 1
        if kend < S:
            pm = jnp.exp2(MASK_LOG2 - m)
            l = l + pm * float(S - kend)
            o = o + pm * jnp.sum(v_tail[u, i], axis=0, keepdims=True)
        inv = pltpu.reciprocal(l, full_range=False)
        ctx_v[h, i * B2:(i + 1) * B2, :] = _pack(o * inv)


def _kernel(x_hbm, ckv_hbm, wq_hbm, wuk_hbm, wuv_hbm, wo_hbm, wr_hbm, wgt_hbm,
            wut_hbm, wd_hbm, c_hbm, wmod_hbm, out_hbm,
            x_v, ckv_v, wq_raw, wkv_raw, wo_v, wgut_v, wgu_v, wd_v, wmod_v,
            a_v, h_v, wq_v, vsum_v, kv_v, ctx_v, x1_v, h2_v, out_v, pend_v, scol_v, mod_v,
            c_v, wr_v,
            sems):
    S, M = x_v.shape
    DC = ckv_v.shape[1]
    H, _, D = ctx_v.shape
    F = wd_v.shape[0]
    NF = wgu_v.shape[1]
    NG = H // HG
    NB = S // BQ
    B2 = BQ // 2
    NA = 4 * NG
    NM = M // 128
    NL = NA // 2
    N0 = NA - NL - NM
    MOD0 = 4

    def kv_half(n):
        g, rows = n // 2, pl.ds((n % 2) * (DC // 2), DC // 2)
        src = wuk_hbm if g < NG else wuv_hbm
        return src.at[rows, pl.ds((g % NG) * HG, HG), :], wkv_raw.at[g, rows]

    def row_slab(src, dst, n, j):
        return src.at[pl.ds(j * n, n)], dst.at[pl.ds(j * n, n)]

    needs = []
    for n in range(NA):
        pairs = [row_slab(ckv_hbm, ckv_v, S // 2, n)] if n < 2 else []
        if n == 1:
            pairs.append(kv_half(2))
        if n and n + 2 < NA:
            pairs.append(kv_half(n + 2))
        if n == N0:
            pairs += [(wq_hbm.at[:, pl.ds(g * HG, HG), :], wq_raw.at[g]) for g in range(NG)]
        if N0 <= n < N0 + NM:
            pairs.append(row_slab(wmod_hbm, wmod_v, 128, n - N0))
        if n == N0 + NM:
            pairs.append((x_hbm, x_v))
        needs.append(pairs)
    needs.append([(wo_hbm, wo_v), (wr_hbm, wr_v)])
    needs.append([(wgt_hbm, wgut_v.at[0, pl.ds(0, F)]), (wut_hbm, wgut_v.at[1, pl.ds(0, F)]),
                  (wd_hbm, wd_v)])
    needs = [[pltpu.make_async_copy(src, dst, sems.at[k % 3]) for src, dst in pairs]
             for k, pairs in enumerate(needs)]
    cp_c = pltpu.make_async_copy(c_hbm, c_v, sems.at[3])
    cp_kv = [pltpu.make_async_copy(*kv_half(n), sems.at[1 + n]) for n in range(2)]
    for cp in [cp_c] + cp_kv + needs[0]:
        cp.start()

    pend_v[...] = jnp.zeros(pend_v.shape, F32)
    wgut_v[:, F:, :] = jnp.zeros((2, NF * 128 - F, M), BF16)
    cp_c.wait()
    cf = c_v[...].astype(F32)
    scol_v[...] = jnp.broadcast_to(_r(cf * jax.nn.sigmoid(cf)), (128, M)).T

    def stage_kv(src, slab, lo, rows):
        w = wkv_raw[src // 2, _ds((src % 2) * (DC // 2) + lo, rows)]
        w = _pack(w.reshape(rows, HG * D))
        a_v[slab, lo // 2:(lo + rows) // 2, :] = w
        return w

    for n in range(2):
        cp_kv[n].wait()
        stage_kv(n, n, 0, DC // 2)

    def kv_loop(lo, hi, side_job):
        rows = S // 2 // A_STEPS

        def body(n, carry):
            for k in range(lo, hi):
                @pl.when(n == k)
                def _(k=k):
                    for cp in needs[k]:
                        cp.wait()
                    for cp in (needs[1] if k == 0 else []) + needs[k + 2]:
                        cp.start()

            g, half = n // 2, n % 2
            for st in range(A_STEPS):
                r0 = half * (S // 2) + st * rows
                w = jnp.concatenate([a_v[2 * (g % 2)], a_v[2 * (g % 2) + 1]], axis=0)
                kv = _dot(ckv_v[_ds(r0, rows), :], _unpack(w))
                if lo >= NA // 2:
                    for b in range(rows // BQ):
                        tot = functools.reduce(
                            jnp.add, [kv[e:e + 8] for e in range(b * BQ, (b + 1) * BQ, 8)])
                        for j in range(HG):
                            vsum_v[g * HG + j - H, _ds((r0 // BQ + b) * 8, 8), :] = (
                                tot[:, j * D:(j + 1) * D])
                kv = _pack(kv)
                for j in range(HG):
                    kv_v[g * HG + j, _ds(r0 // 2, rows // 2), :] = kv[:, j * D:(j + 1) * D]
            pacer = _Pacer()
            src = jnp.where(n == 0, 0, jnp.minimum(n + 2, NA - 1))
            for r in range(0, DC // 2, ST_ROWS):
                pacer.tick(stage_kv(src, (n + 2) % 4, r, ST_ROWS))
            side_job(n - lo, pacer)
            pacer.idle(END_GAP)
            a_v[MOD0, 64:72, 0:128] = pacer.word
            return carry

        lax.fori_loop(lo, hi, body, 0)

    def mod_and_wq(t, pacer):
        rows = _ds(t * 128, 128)
        tiles = [(i, j) for i in range(6) for j in range(M // 128)]
        for g in range(NG):
            for r in range(0, 128, ST_ROWS):
                if tiles:
                    i, j = tiles.pop(0)
                    prod = wmod_v[rows, i * M + j * 128:i * M + (j + 1) * 128].astype(F32)
                    prod = prod * scol_v[rows, :]
                    acc = functools.reduce(jnp.add, [prod[e:e + 8] for e in range(0, 128, 8)])
                    a_v[MOD0 + t, i * 8:(i + 1) * 8, j * 128:(j + 1) * 128] = (
                        pltpu.bitcast(acc, U32))
                    pacer.tick(acc, 0)
                w = _pack(wq_raw[g, _ds(t * 128 + r, ST_ROWS)].reshape(ST_ROWS, HG * D))
                for j in range(HG):
                    wq_v[g * HG + j, _ds(t * 64 + r // 2, ST_ROWS // 2), :] = (
                        w[:, j * D:(j + 1) * D])
                pacer.tick(w)
        assert not tiles

    def mod_row(i):
        return mod_v[i, 0:1, :]

    def ln1(t, pacer):
        for e in range(S // NL // LN_ROWS):
            r0 = t * (S // NL) + e * LN_ROWS
            xf = x_v[_ds(r0, LN_ROWS), :].astype(F32)
            h = _pack(_modulated_ln(xf, mod_row(0), mod_row(1)))
            h_v[_ds(r0 // 2, LN_ROWS // 2), :] = h
            pacer.tick(h, LN1_GAP)

    def catch_up(t, pacer):
        for r in range(0, DC // 2, ST_ROWS):
            pacer.tick(stage_kv(jnp.where(t == 1, 2, 0), jnp.where(t == 1, 2, MOD0 + 1),
                                r, ST_ROWS))

    kv_loop(0, N0, catch_up)
    kv_loop(N0, N0 + NM, mod_and_wq)
    for i in range(6):
        parts = [pltpu.bitcast(a_v[MOD0 + t, i * 8:(i + 1) * 8, :M], F32)
                 for t in range(NM)]
        mod = _r(jnp.sum(functools.reduce(jnp.add, parts), axis=0, keepdims=True))
        if i % 3 == 1:
            mod = _r(1.0 + mod)
        mod_v[i] = jnp.broadcast_to(mod, (8, M))
    kv_loop(N0 + NM, NA, ln1)

    def heads_body(it, carry):
        _attention(it * HEADS_PER_ITER, h_v, wq_v, kv_v, vsum_v, ctx_v)
        return carry

    lax.fori_loop(0, H // HEADS_PER_ITER, heads_body, 0)

    for cp in needs[NA] + needs[NA + 1]:
        cp.wait()
    wr = wr_v[...].astype(F32).reshape(1, M)

    def out_copy(blk):
        return pltpu.make_async_copy(out_v.at[_ds(blk * BQ, BQ), :],
                                     out_hbm.at[_ds(blk * BQ, BQ), :], sems.at[3])

    def finish_rows(attn, r0, scores):
        n = attn.shape[0]
        rows = _ds(r0, n)
        x1 = _r(x_v[rows, :].astype(F32) + _r(mod_row(2) * _r(attn)))
        h2 = _modulated_ln(x1, mod_row(3), mod_row(4))
        out = x1 + _r(mod_row(5) * (h2 + h2 * 0.0))
        x1_v[rows, :] = x1.astype(BF16)
        h2_v[rows, :] = h2.astype(BF16)
        out = out.astype(BF16)
        out_v[rows, :] = out
        r = jnp.sum(h2 * wr, axis=1, keepdims=True)
        lane = lax.broadcasted_iota(I32, scores.shape, 1)
        for g in range(n // 8):
            scores = jnp.where(lane == r0 // 8 + g, r[g * 8:(g + 1) * 8], scores)
        return scores, out

    def c_body(t, scores):
        prev_blk = jnp.maximum(t * SUB_C - 1, 0)
        attn = pend_v[...]
        pacer = _Pacer()
        for b in range(SUB_C):
            blk = t * SUB_C + b
            f = jnp.minimum(blk, NF - 1)
            for e in range(2):
                w = _pack(wgut_v[e, _ds(f * 128, 128), :].T)
                wgu_v[e, f] = w
                pacer.tick(w)
            for lo in range(0, BQ, LN_ROWS):
                scores, out = finish_rows(attn[lo:lo + LN_ROWS], prev_blk * BQ + lo, scores)
                pacer.tick(scores, 0)
                pacer.tick(out, LN2_GAP)
            ctx = jnp.concatenate([ctx_v[h, _ds(blk * B2, B2), :] for h in range(H)], axis=1)
            attn = _dot(_unpack(ctx), wo_v[...])
            prev_blk = blk
        pend_v[...] = attn
        a_v[MOD0, 64:72, 0:128] = pacer.word

        @pl.when(t > 0)
        def _():
            out_copy(t * SUB_C - 1).start()

        for b in range(SUB_C - 1):
            out_copy(t * SUB_C + b).start()
        return scores

    scores = jnp.zeros((8, S // 8), F32)
    scores = lax.fori_loop(0, NB // SUB_C, c_body, scores)
    scores, _ = finish_rows(pend_v[...], (NB - 1) * BQ, scores)

    rb = _r(scores)
    bits = pltpu.bitcast(jnp.where(rb == 0.0, 0.0, rb), I32)
    k16 = (bits >> 16) & 0xFFFF
    k16 = jnp.where(bits < 0, 0xFFFF - k16, k16 + 0x8000)
    k16 = jnp.where(rb != rb, 0, k16)
    ridx = (lax.broadcasted_iota(I32, scores.shape, 1) * 8
            + lax.broadcasted_iota(I32, scores.shape, 0))
    idx_bits = (S - 1).bit_length()
    key = pltpu.bitcast((k16 << idx_bits) + (S - 1 - ridx) + (1 << 29), F32)
    picks = []
    for _ in range(TOPK):
        top = jnp.max(jnp.max(key, axis=1, keepdims=True), axis=0, keepdims=True)
        key = jnp.where(key == top, 1.0e-30, key)
        picks.append(S - 1 - (pltpu.bitcast(top, I32)[0, 0] & ((1 << idx_bits) - 1)))

    row16 = lax.broadcasted_iota(I32, (16, M), 0)

    def tile_of(i):
        return _ds((i // 16) * 16, 16)

    sel = jnp.zeros((16, M), F32)
    for j, i in enumerate(picks):
        tile = h2_v[tile_of(i), :].astype(F32)
        hrow = jnp.sum(jnp.where(row16 == i % 16, tile, 0.0), axis=0, keepdims=True)
        sel = jnp.where(row16 == j, hrow, sel)

    sel_b = sel.astype(BF16)
    g, u = [
        _r(_dot(sel_b, _unpack(jnp.concatenate([wgu_v[e, f] for f in range(NF)], axis=1))))
        for e in range(2)]
    g = _r(g * jax.nn.sigmoid(g))
    y = _r(_dot((g * u).astype(BF16)[:, :F], wd_v[...]))
    gate = _r(jax.nn.sigmoid(_r(jnp.sum(sel * wr, axis=1, keepdims=True))))
    y = _r(y * gate)
    delta = _r(mod_row(5) * _r(sel + _r(sel * 0.0 + y)))

    for t in range(NB - 1):
        out_copy(t).wait()
    for j, i in enumerate(picks):
        new = (x1_v[tile_of(i), :].astype(F32) + delta[j:j + 1, :]).astype(BF16)
        out_v[tile_of(i), :] = jnp.where(row16 == i % 16, new, out_v[tile_of(i), :])

    def fix_copy(j):
        return pltpu.make_async_copy(out_v.at[tile_of(picks[j]), :],
                                     out_hbm.at[tile_of(picks[j]), :], sems.at[3])

    first = []
    for j in range(TOPK):
        f = picks[j] < (NB - 1) * BQ
        for e in range(j):
            f = jnp.logical_and(f, picks[e] // 16 != picks[j] // 16)
        first.append(f)
    out_copy(NB - 1).start()
    for j in range(TOPK):
        pl.when(first[j])(fix_copy(j).start)
    out_copy(NB - 1).wait()
    for j in range(TOPK):
        pl.when(first[j])(fix_copy(j).wait)


@jax.jit
def pallas_adaLN_cond__compressed_kv_cla__moe_arch_mod__prompt_kernel(
    A_x: jax.Array,
    A_c_kv: jax.Array,
    A_w_q: jax.Array,
    A_w_uk: jax.Array,
    A_w_uv: jax.Array,
    A_w_o: jax.Array,
    B_x: jax.Array,
    B_w_r: jax.Array,
    B_w_gate: jax.Array,
    B_w_up: jax.Array,
    B_w_down: jax.Array,
    c: jax.Array,
    w_mod: jax.Array,
):
    del B_x
    _, S, M = A_x.shape
    DC = A_c_kv.shape[2]
    _, H, D = A_w_q.shape
    F = B_w_gate.shape[1]
    NF = pl.cdiv(F, 128)
    NG = H // HG

    hbm = pl.BlockSpec(memory_space=pl.ANY)
    scratch = [
        pltpu.VMEM((S, M), BF16),
        pltpu.VMEM((S, DC), BF16),
        pltpu.VMEM((NG, M, HG, D), BF16),
        pltpu.VMEM((2 * NG, DC, HG, D), BF16),
        pltpu.VMEM((H * D, M), BF16),
        pltpu.VMEM((2, NF * 128, M), BF16),
        pltpu.VMEM((2, NF, M // 2, 128), U32),
        pltpu.VMEM((F, M), BF16),
        pltpu.VMEM((M, 6 * M), BF16),
        pltpu.VMEM((4 + M // 128, DC // 4, HG * D), U32),
        pltpu.VMEM((S // 2, M), U32),
        pltpu.VMEM((H, M // 2, D), U32),
        pltpu.VMEM((H, S // BQ * 8, D), F32),
        pltpu.VMEM((2 * H, S // 2, D), U32),
        pltpu.VMEM((H, S // 2, D), U32),
        pltpu.VMEM((S, M), BF16),
        pltpu.VMEM((S, M), BF16),
        pltpu.VMEM((S, M), BF16),
        pltpu.VMEM((BQ, M), F32),
        pltpu.VMEM((M, 128), F32),
        pltpu.VMEM((6, 8, M), F32),
        pltpu.VMEM((1, M), BF16),
        pltpu.VMEM((M,), BF16),
        pltpu.SemaphoreType.DMA((4,)),
    ]
    out = pl.pallas_call(
        _kernel,
        in_specs=[hbm] * 12,
        out_specs=hbm,
        out_shape=jax.ShapeDtypeStruct((S, M), A_x.dtype),
        scratch_shapes=scratch,
        compiler_params=pltpu.CompilerParams(vmem_limit_bytes=124 * 1024 * 1024),
        name="adaln_cla_moe",
    )(A_x.reshape(S, M), A_c_kv.reshape(S, DC), A_w_q, A_w_uk, A_w_uv,
      A_w_o.reshape(H * D, M), B_w_r, B_w_gate.T, B_w_up.T, B_w_down, c, w_mod)
    return out.reshape(A_x.shape)
```

```python
import functools
import math

import jax
import jax.numpy as jnp
from jax import lax
import jax.experimental.pallas as pl
import jax.experimental.pallas.tpu as pltpu

F32 = jnp.float32
BF16 = jnp.bfloat16
U32 = jnp.uint32
I32 = jnp.int32

TOPK = 8
EPS = 1e-05
LOG2E = math.log2(math.e)
MASK_LOG2 = -1000000000.0 * LOG2E
BQ = 128
N_MXU = 4
HG = 8
A_STEPS = 2
HEADS_PER_ITER = 2
SUB_C = 2
LN_ROWS = 16
ST_ROWS = 16
LN1_GAP = 2
LN2_GAP = 4
END_GAP = 2
EXP_ROWS = 16
NT = (((1,), (1,)), ((), ()))


def _r(x):
    return x.astype(BF16).astype(F32)


def _sigmoid(x):
    return _r(1.0 / _r(1.0 + _r(jnp.exp(-x))))


def _dot(a, b):
    return jnp.dot(a, b, preferred_element_type=F32)


def _dot_nt(a, b):
    return lax.dot_general(a, b, NT, preferred_element_type=F32)


def _pack(x):
    return pltpu.bitcast(x.astype(BF16), U32)


def _unpack(x):
    return pltpu.bitcast(x, BF16)


def _ds(start, size):
    if not isinstance(start, int):
        start = pl.multiple_of(start, size)
    return pl.ds(start, size)


class _Pacer:
    def __init__(self):
        self.word = None

    def tick(self, x, gap=1):
        x = pltpu.bitcast(x, U32)
        tiles = [x[r:r + 8, c:c + 128]
                 for r in range(0, x.shape[0], 8) for c in range(0, x.shape[1], 128)]
        word = functools.reduce(jnp.bitwise_or, tiles)
        self.word = word if self.word is None else self.word | word
        self.idle(gap)

    def idle(self, gap):
        for _ in range(gap):
            self.word = pltpu.roll(self.word, 1, 1)


def _modulated_ln(x, shift, scale1):
    inv_n = 1.0 / x.shape[-1]
    mean = jnp.sum(x, axis=-1, keepdims=True) * inv_n
    xc = x - mean
    var = jnp.sum(xc * xc, axis=-1, keepdims=True) * inv_n
    std = _r(jnp.sqrt(_r(_r(var) + EPS)))
    n = _r(_r(x - _r(mean)) / std)
    return _r(_r(n * scale1) + shift)


def _attention(h0, h_v, wq_v, kv_v, vsum_v, ctx_v):
    H, B2, D = ctx_v.shape[0], BQ // 2, ctx_v.shape[2]
    S = 2 * ctx_v.shape[1]
    NB = S // BQ
    causal = (lax.broadcasted_iota(I32, (BQ, BQ), 1)
              <= lax.broadcasted_iota(I32, (BQ, BQ), 0))
    v_tail = {}
    for u in range(HEADS_PER_ITER):
        tot = None
        for i in range(NB - 1, 0, -1):
            part = vsum_v[h0 + u, i * 8:(i + 1) * 8, :]
            tot = part if tot is None else tot + part
            v_tail[u, i - 1] = tot

    steps = [(u, i) for u in range(HEADS_PER_ITER) for i in range(NB)]
    plan = [("q", *steps[0]), ("q", *steps[1]), ("s", *steps[0])]
    for t, step in enumerate(steps):
        plan += [("q", *st) for st in steps[t + 2:t + 3]]
        plan += [("s", *st) for st in steps[t + 1:t + 2]]
        plan.append(("o", *step))

    qs, scores = {}, {}
    tiles = 0
    inv = None
    for op, u, i in plan:
        h = h0 + u
        kend = (i + 1) * BQ
        if op == "q":
            q = _dot(_unpack(h_v[i * B2:(i + 1) * B2, :]), _unpack(wq_v[h]))
            qs[u, i] = (q * (D ** (-0.5) * LOG2E)).astype(BF16)
            tiles += h_v.shape[1] // 128
            continue
        if op == "s":
            s = _dot_nt(qs[u, i], _unpack(kv_v[h, :kend // 2, :]))
            sd = jnp.where(causal, s[:, kend - BQ:], MASK_LOG2)
            s = jnp.concatenate([s[:, :kend - BQ], sd], axis=1) if i else sd
            m = functools.reduce(jnp.maximum,
                                 [s[:, c:c + 128] for c in range(0, kend, 128)])
            if kend < S:
                m = jnp.concatenate([m[:-8], jnp.maximum(m[-8:], MASK_LOG2)], axis=0)
            scores[u, i] = s, jnp.max(m, axis=1, keepdims=True)
            tiles += i + 1
            continue
        s, m = scores[u, i]
        if inv is not None:
            m = jnp.where(inv < 0.0, inv, m)
        mb = jnp.broadcast_to(m, (BQ, 128))
        ps, ls, last = [], [None] * (BQ // EXP_ROWS), None
        lo, hi = 0, min(kend, (N_MXU - tiles % N_MXU) * BQ)
        while lo < kend:
            rows = []
            for e in range(BQ // EXP_ROWS):
                r = slice(e * EXP_ROWS, (e + 1) * EXP_ROWS)
                me = mb[r] if last is None else jnp.where(last < 0.0, last, mb[r])
                p = [jnp.exp2(s[r, c:c + 128] - me) for c in range(lo, hi, 128)]
                ls[e] = last = functools.reduce(
                    jnp.add, p if ls[e] is None else [ls[e]] + p)
                rows.append(jnp.concatenate(p, axis=1).astype(BF16))
            ps.append(jnp.concatenate(rows, axis=0))
            lo, hi = hi, min(kend, hi + N_MXU * BQ)
        l = jnp.sum(jnp.concatenate(ls, axis=0), axis=1, keepdims=True)
        o = _dot(jnp.concatenate(ps, axis=1), _unpack(kv_v[H + h, :kend // 2, :]))
        tiles += i + 1
        if kend < S:
            pm = jnp.exp2(MASK_LOG2 - m)
            l = l + pm * float(S - kend)
            o = o + pm * jnp.sum(v_tail[u, i], axis=0, keepdims=True)
        inv = pltpu.reciprocal(l, full_range=False)
        ctx_v[h, i * B2:(i + 1) * B2, :] = _pack(o * inv)


def _kernel(x_hbm, ckv_hbm, wq_hbm, wuk_hbm, wuv_hbm, wo_hbm, wr_hbm, wgt_hbm,
            wut_hbm, wd_hbm, c_hbm, wmod_hbm, out_hbm,
            x_v, ckv_v, wq_raw, wkv_raw, wo_v, wgut_v, wgu_v, wd_v, wmod_v,
            a_v, h_v, wq_v, vsum_v, kv_v, ctx_v, x1_v, h2_v, out_v, pend_v, scol_v, mod_v,
            c_v, wr_v,
            sems):
    S, M = x_v.shape
    DC = ckv_v.shape[1]
    H, _, D = ctx_v.shape
    F = wd_v.shape[0]
    NF = wgu_v.shape[1]
    NG = H // HG
    NB = S // BQ
    B2 = BQ // 2
    NA = 4 * NG
    NM = M // 128
    NL = NA // 2
    N0 = NA - NL - NM
    MOD0 = 4

    def kv_half(n):
        g, rows = n // 2, pl.ds((n % 2) * (DC // 2), DC // 2)
        src = wuk_hbm if g < NG else wuv_hbm
        return src.at[rows, pl.ds((g % NG) * HG, HG), :], wkv_raw.at[g, rows]

    def row_slab(src, dst, n, j):
        return src.at[pl.ds(j * n, n)], dst.at[pl.ds(j * n, n)]

    needs = []
    for n in range(NA):
        pairs = [row_slab(ckv_hbm, ckv_v, S // 2, n)] if n < 2 else []
        if n == 1:
            pairs.append(kv_half(2))
        if n and n + 2 < NA:
            pairs.append(kv_half(n + 2))
        if n == N0:
            pairs += [(wq_hbm.at[:, pl.ds(g * HG, HG), :], wq_raw.at[g]) for g in range(NG)]
        if N0 <= n < N0 + NM:
            pairs.append(row_slab(wmod_hbm, wmod_v, 128, n - N0))
        if n == N0 + NM:
            pairs.append((x_hbm, x_v))
        needs.append(pairs)
    needs.append([(wo_hbm, wo_v), (wr_hbm, wr_v)])
    needs.append([(wgt_hbm, wgut_v.at[0, pl.ds(0, F)]), (wut_hbm, wgut_v.at[1, pl.ds(0, F)]),
                  (wd_hbm, wd_v)])
    needs = [[pltpu.make_async_copy(src, dst, sems.at[k % 3]) for src, dst in pairs]
             for k, pairs in enumerate(needs)]
    cp_c = pltpu.make_async_copy(c_hbm, c_v, sems.at[3])
    cp_kv = [pltpu.make_async_copy(*kv_half(n), sems.at[1 + n]) for n in range(2)]
    for cp in [cp_c] + cp_kv + needs[0]:
        cp.start()

    pend_v[...] = jnp.zeros(pend_v.shape, F32)
    wgut_v[:, F:, :] = jnp.zeros((2, NF * 128 - F, M), BF16)
    cp_c.wait()
    cf = c_v[...].astype(F32)
    scol_v[...] = jnp.broadcast_to(_r(cf * _sigmoid(cf)), (128, M)).T

    def stage_kv(src, slab, lo, rows):
        w = wkv_raw[src // 2, _ds((src % 2) * (DC // 2) + lo, rows)]
        w = _pack(w.reshape(rows, HG * D))
        a_v[slab, lo // 2:(lo + rows) // 2, :] = w
        return w

    for n in range(2):
        cp_kv[n].wait()
        stage_kv(n, n, 0, DC // 2)

    def kv_loop(lo, hi, side_job):
        rows = S // 2 // A_STEPS

        def body(n, carry):
            for k in range(lo, hi):
                @pl.when(n == k)
                def _(k=k):
                    for cp in needs[k]:
                        cp.wait()
                    for cp in (needs[1] if k == 0 else []) + needs[k + 2]:
                        cp.start()

            g, half = n // 2, n % 2
            for st in range(A_STEPS):
                r0 = half * (S // 2) + st * rows
                w = jnp.concatenate([a_v[2 * (g % 2)], a_v[2 * (g % 2) + 1]], axis=0)
                kv = _dot(ckv_v[_ds(r0, rows), :], _unpack(w))
                if lo >= NA // 2:
                    for b in range(rows // BQ):
                        tot = functools.reduce(
                            jnp.add, [kv[e:e + 8] for e in range(b * BQ, (b + 1) * BQ, 8)])
                        for j in range(HG):
                            vsum_v[g * HG + j - H, _ds((r0 // BQ + b) * 8, 8), :] = (
                                tot[:, j * D:(j + 1) * D])
                kv = _pack(kv)
                for j in range(HG):
                    kv_v[g * HG + j, _ds(r0 // 2, rows // 2), :] = kv[:, j * D:(j + 1) * D]
            pacer = _Pacer()
            src = jnp.where(n == 0, 0, jnp.minimum(n + 2, NA - 1))
            for r in range(0, DC // 2, ST_ROWS):
                pacer.tick(stage_kv(src, (n + 2) % 4, r, ST_ROWS))
            side_job(n - lo, pacer)
            pacer.idle(END_GAP)
            a_v[MOD0, 64:72, 0:128] = pacer.word
            return carry

        lax.fori_loop(lo, hi, body, 0)

    def mod_and_wq(t, pacer):
        rows = _ds(t * 128, 128)
        tiles = [(i, j) for i in range(6) for j in range(M // 128)]
        for g in range(NG):
            for r in range(0, 128, ST_ROWS):
                if tiles:
                    i, j = tiles.pop(0)
                    prod = wmod_v[rows, i * M + j * 128:i * M + (j + 1) * 128].astype(F32)
                    prod = prod * scol_v[rows, :]
                    acc = functools.reduce(jnp.add, [prod[e:e + 8] for e in range(0, 128, 8)])
                    a_v[MOD0 + t, i * 8:(i + 1) * 8, j * 128:(j + 1) * 128] = (
                        pltpu.bitcast(acc, U32))
                    pacer.tick(acc, 0)
                w = _pack(wq_raw[g, _ds(t * 128 + r, ST_ROWS)].reshape(ST_ROWS, HG * D))
                for j in range(HG):
                    wq_v[g * HG + j, _ds(t * 64 + r // 2, ST_ROWS // 2), :] = (
                        w[:, j * D:(j + 1) * D])
                pacer.tick(w)
        assert not tiles

    def mod_row(i):
        return mod_v[i, 0:1, :]

    def ln1(t, pacer):
        for e in range(S // NL // LN_ROWS):
            r0 = t * (S // NL) + e * LN_ROWS
            xf = x_v[_ds(r0, LN_ROWS), :].astype(F32)
            h = _pack(_modulated_ln(xf, mod_row(0), mod_row(1)))
            h_v[_ds(r0 // 2, LN_ROWS // 2), :] = h
            pacer.tick(h, LN1_GAP)

    def catch_up(t, pacer):
        for r in range(0, DC // 2, ST_ROWS):
            pacer.tick(stage_kv(jnp.where(t == 1, 2, 0), jnp.where(t == 1, 2, MOD0 + 1),
                                r, ST_ROWS))

    kv_loop(0, N0, catch_up)
    kv_loop(N0, N0 + NM, mod_and_wq)
    for i in range(6):
        parts = [pltpu.bitcast(a_v[MOD0 + t, i * 8:(i + 1) * 8, :M], F32)
                 for t in range(NM)]
        mod = _r(jnp.sum(functools.reduce(jnp.add, parts), axis=0, keepdims=True))
        if i % 3 == 1:
            mod = _r(1.0 + mod)
        mod_v[i] = jnp.broadcast_to(mod, (8, M))
    kv_loop(N0 + NM, NA, ln1)

    def heads_body(it, carry):
        _attention(it * HEADS_PER_ITER, h_v, wq_v, kv_v, vsum_v, ctx_v)
        return carry

    lax.fori_loop(0, H // HEADS_PER_ITER, heads_body, 0)

    for cp in needs[NA] + needs[NA + 1]:
        cp.wait()
    wr = wr_v[...].astype(F32).reshape(1, M)

    def out_copy(blk):
        return pltpu.make_async_copy(out_v.at[_ds(blk * BQ, BQ), :],
                                     out_hbm.at[_ds(blk * BQ, BQ), :], sems.at[3])

    def finish_rows(attn, r0, scores):
        n = attn.shape[0]
        rows = _ds(r0, n)
        x1 = _r(x_v[rows, :].astype(F32) + _r(mod_row(2) * _r(attn)))
        h2 = _modulated_ln(x1, mod_row(3), mod_row(4))
        out = x1 + _r(mod_row(5) * (h2 + h2 * 0.0))
        x1_v[rows, :] = x1.astype(BF16)
        h2_v[rows, :] = h2.astype(BF16)
        out = out.astype(BF16)
        out_v[rows, :] = out
        r = jnp.sum(h2 * wr, axis=1, keepdims=True)
        lane = lax.broadcasted_iota(I32, scores.shape, 1)
        for g in range(n // 8):
            scores = jnp.where(lane == r0 // 8 + g, r[g * 8:(g + 1) * 8], scores)
        return scores, out

    def c_body(t, scores):
        prev_blk = jnp.maximum(t * SUB_C - 1, 0)
        attn = pend_v[...]
        pacer = _Pacer()
        for b in range(SUB_C):
            blk = t * SUB_C + b
            f = jnp.minimum(blk, NF - 1)
            for e in range(2):
                w = _pack(wgut_v[e, _ds(f * 128, 128), :].T)
                wgu_v[e, f] = w
                pacer.tick(w)
            for lo in range(0, BQ, LN_ROWS):
                scores, out = finish_rows(attn[lo:lo + LN_ROWS], prev_blk * BQ + lo, scores)
                pacer.tick(scores, 0)
                pacer.tick(out, LN2_GAP)
            ctx = jnp.concatenate([ctx_v[h, _ds(blk * B2, B2), :] for h in range(H)], axis=1)
            attn = _dot(_unpack(ctx), wo_v[...])
            prev_blk = blk
        pend_v[...] = attn
        a_v[MOD0, 64:72, 0:128] = pacer.word

        @pl.when(t > 0)
        def _():
            out_copy(t * SUB_C - 1).start()

        for b in range(SUB_C - 1):
            out_copy(t * SUB_C + b).start()
        return scores

    scores = jnp.zeros((8, S // 8), F32)
    scores = lax.fori_loop(0, NB // SUB_C, c_body, scores)
    scores, _ = finish_rows(pend_v[...], (NB - 1) * BQ, scores)

    rb = _r(scores)
    bits = pltpu.bitcast(jnp.where(rb == 0.0, 0.0, rb), I32)
    k16 = (bits >> 16) & 0xFFFF
    k16 = jnp.where(bits < 0, 0xFFFF - k16, k16 + 0x8000)
    k16 = jnp.where(rb != rb, 0, k16)
    ridx = (lax.broadcasted_iota(I32, scores.shape, 1) * 8
            + lax.broadcasted_iota(I32, scores.shape, 0))
    idx_bits = (S - 1).bit_length()
    key = pltpu.bitcast((k16 << idx_bits) + (S - 1 - ridx) + (1 << 29), F32)
    picks = []
    for _ in range(TOPK):
        top = jnp.max(jnp.max(key, axis=1, keepdims=True), axis=0, keepdims=True)
        key = jnp.where(key == top, 1.0e-30, key)
        picks.append(S - 1 - (pltpu.bitcast(top, I32)[0, 0] & ((1 << idx_bits) - 1)))

    row16 = lax.broadcasted_iota(I32, (16, M), 0)

    def tile_of(i):
        return _ds((i // 16) * 16, 16)

    sel = jnp.zeros((16, M), F32)
    for j, i in enumerate(picks):
        tile = h2_v[tile_of(i), :].astype(F32)
        hrow = jnp.sum(jnp.where(row16 == i % 16, tile, 0.0), axis=0, keepdims=True)
        sel = jnp.where(row16 == j, hrow, sel)

    sel_b = sel.astype(BF16)
    g, u = [
        _r(_dot(sel_b, _unpack(jnp.concatenate([wgu_v[e, f] for f in range(NF)], axis=1))))
        for e in range(2)]
    g = _r(g * _sigmoid(g))
    y = _r(_dot((g * u).astype(BF16)[:, :F], wd_v[...]))
    gate = _sigmoid(_r(jnp.sum(sel * wr, axis=1, keepdims=True)))
    y = _r(y * gate)
    delta = _r(mod_row(5) * _r(sel + _r(sel * 0.0 + y)))

    for t in range(NB - 1):
        out_copy(t).wait()
    for j, i in enumerate(picks):
        new = (x1_v[tile_of(i), :].astype(F32) + delta[j:j + 1, :]).astype(BF16)
        out_v[tile_of(i), :] = jnp.where(row16 == i % 16, new, out_v[tile_of(i), :])

    def fix_copy(j):
        return pltpu.make_async_copy(out_v.at[tile_of(picks[j]), :],
                                     out_hbm.at[tile_of(picks[j]), :], sems.at[3])

    first = []
    for j in range(TOPK):
        f = picks[j] < (NB - 1) * BQ
        for e in range(j):
            f = jnp.logical_and(f, picks[e] // 16 != picks[j] // 16)
        first.append(f)
    out_copy(NB - 1).start()
    for j in range(TOPK):
        pl.when(first[j])(fix_copy(j).start)
    out_copy(NB - 1).wait()
    for j in range(TOPK):
        pl.when(first[j])(fix_copy(j).wait)


@jax.jit
def pallas_adaLN_cond__compressed_kv_cla__moe_arch_mod__prompt_kernel(
    A_x: jax.Array,
    A_c_kv: jax.Array,
    A_w_q: jax.Array,
    A_w_uk: jax.Array,
    A_w_uv: jax.Array,
    A_w_o: jax.Array,
    B_x: jax.Array,
    B_w_r: jax.Array,
    B_w_gate: jax.Array,
    B_w_up: jax.Array,
    B_w_down: jax.Array,
    c: jax.Array,
    w_mod: jax.Array,
):
    del B_x
    _, S, M = A_x.shape
    DC = A_c_kv.shape[2]
    _, H, D = A_w_q.shape
    F = B_w_gate.shape[1]
    NF = pl.cdiv(F, 128)
    NG = H // HG

    hbm = pl.BlockSpec(memory_space=pl.ANY)
    scratch = [
        pltpu.VMEM((S, M), BF16),
        pltpu.VMEM((S, DC), BF16),
        pltpu.VMEM((NG, M, HG, D), BF16),
        pltpu.VMEM((2 * NG, DC, HG, D), BF16),
        pltpu.VMEM((H * D, M), BF16),
        pltpu.VMEM((2, NF * 128, M), BF16),
        pltpu.VMEM((2, NF, M // 2, 128), U32),
        pltpu.VMEM((F, M), BF16),
        pltpu.VMEM((M, 6 * M), BF16),
        pltpu.VMEM((4 + M // 128, DC // 4, HG * D), U32),
        pltpu.VMEM((S // 2, M), U32),
        pltpu.VMEM((H, M // 2, D), U32),
        pltpu.VMEM((H, S // BQ * 8, D), F32),
        pltpu.VMEM((2 * H, S // 2, D), U32),
        pltpu.VMEM((H, S // 2, D), U32),
        pltpu.VMEM((S, M), BF16),
        pltpu.VMEM((S, M), BF16),
        pltpu.VMEM((S, M), BF16),
        pltpu.VMEM((BQ, M), F32),
        pltpu.VMEM((M, 128), F32),
        pltpu.VMEM((6, 8, M), F32),
        pltpu.VMEM((1, M), BF16),
        pltpu.VMEM((M,), BF16),
        pltpu.SemaphoreType.DMA((4,)),
    ]
    out = pl.pallas_call(
        _kernel,
        in_specs=[hbm] * 12,
        out_specs=hbm,
        out_shape=jax.ShapeDtypeStruct((S, M), A_x.dtype),
        scratch_shapes=scratch,
        compiler_params=pltpu.CompilerParams(vmem_limit_bytes=124 * 1024 * 1024),
        name="adaln_cla_moe",
    )(A_x.reshape(S, M), A_c_kv.reshape(S, DC), A_w_q, A_w_uk, A_w_uv,
      A_w_o.reshape(H * D, M), B_w_r, B_w_gate.T, B_w_up.T, B_w_down, c, w_mod)
    return out.reshape(A_x.shape)
```
